```python
import jax
import jax.numpy as jnp

def _softmax(x, axis=-1):
    return jax.nn.softmax(x, axis=axis)

def _gelu(x):
    return jax.nn.gelu(x, approximate=True)

def _silu(x):
    return jax.nn.silu(x)

def _sigmoid(x):
    return jax.nn.sigmoid(x)

def _layernorm(x, axis=-1, eps=1e-05):
    m = jnp.mean(x, axis=axis, keepdims=True)
    v = jnp.var(x, axis=axis, keepdims=True)
    return (x - m) / jnp.sqrt(v + eps)

def _scatter_add(tgt, idx, src, axis=0):
    return tgt.at[idx].add(src)

def _segment_sum(src, seg, n):
    return jax.ops.segment_sum(src, seg, n)

class _Rng:

    def __init__(self, key):
        self._k = key

    def _next(self):
        self._k, sub = jax.random.split(self._k)
        return sub

    def normal(self, shape):
        return jax.random.normal(self._next(), shape, dtype=jnp.bfloat16)

    def randint(self, lo, hi, shape):
        return jax.random.randint(self._next(), shape, lo, hi, dtype=jnp.int32)

    def uniform(self, shape, lo=0.0, hi=1.0):
        return jax.random.uniform(self._next(), shape, jnp.bfloat16, lo, hi)

    def permutation(self, n):
        return jax.random.permutation(self._next(), n)
kernel_name = 'adaLN_cond__sliding_block_cached__moe_arch_mod__decode'

def setup_inputs():
    _rng = _Rng(jax.random.key(int.from_bytes(__import__("os").urandom(4), "little")))
    _w = lambda a: (lambda t: t.astype(jnp.bfloat16) if jnp.issubdtype(t.dtype, jnp.floating) else t)(jnp.asarray(a))

    def _A_setup():
        B, Sq, D = (8, 1, 576)
        Hq, Hkv, Sk, Dh = (32, 16, 8192, 128)
        assert Hq % Hkv == 0, (Hq, Hkv)
        return {'x': _w((lambda *s: _rng.normal(s) * 0.05)(B, Sq, D)), 'k_cache': _w((lambda *s: _rng.normal(s) * 0.05)(B, Hkv, Sk, Dh)), 'v_cache': _w((lambda *s: _rng.normal(s) * 0.05)(B, Hkv, Sk, Dh)), 'wq': _w((lambda *s: _rng.normal(s) * 0.05)(D, Hq * Dh) * D ** (-0.5)), 'wo': _w((lambda *s: _rng.normal(s) * 0.05)(Hq * Dh, D) * (Hq * Dh) ** (-0.5))}
    _A_in = _A_setup()

    def _B_setup():
        B, S, D, F, C = (8, 1, 576, 4608, 1)
        return {'x': _w((lambda *s: _rng.normal(s) * 0.05)(B, S, D)), 'w_r': _w((lambda *s: _rng.normal(s) * 0.05)(D)), 'w_gate': _w((lambda *s: _rng.normal(s) * 0.05)(D, F)), 'w_up': _w((lambda *s: _rng.normal(s) * 0.05)(D, F)), 'w_down': _w((lambda *s: _rng.normal(s) * 0.05)(F, D))}
    _B_in = _B_setup()
    return {'A_x': _A_in['x'], 'A_k_cache': _A_in['k_cache'], 'A_v_cache': _A_in['v_cache'], 'A_wq': _A_in['wq'], 'A_wo': _A_in['wo'], 'B_x': _B_in['x'], 'B_w_r': _B_in['w_r'], 'B_w_gate': _B_in['w_gate'], 'B_w_up': _B_in['w_up'], 'B_w_down': _B_in['w_down'], 'c': _w((lambda *s: _rng.normal(s) * 0.05)(8, 576)), 'w_mod': _w((lambda *s: _rng.normal(s) * 0.05)(576, 6 * 576) * 576 ** (-0.5))}

def reference(A_x, A_k_cache, A_v_cache, A_wq, A_wo, B_x, B_w_r, B_w_gate, B_w_up, B_w_down, c, w_mod):

    def _A_ref(x, k_cache, v_cache, wq, wo):
        B, Sq, D = x.shape
        Hq, Dh = (32, 128)
        Hkv, Sk = (k_cache.shape[1], k_cache.shape[2])
        W = min(4096, max(256, Sk // 4))
        rep = Hq // Hkv
        q = (lambda x, *d: x.transpose(*d))((x @ wq).reshape(B, Sq, Hq, Dh), 0, 2, 1, 3)
        k = jnp.repeat(k_cache[:, :, Sk - W:, :], rep, axis=1)
        v = jnp.repeat(v_cache[:, :, Sk - W:, :], rep, axis=1)
        scores = jnp.einsum('bhqd,bhkd->bhqk', q, k) * Dh ** (-0.5)
        p = _softmax(scores, axis=-1)
        o = jnp.einsum('bhqk,bhkd->bhqd', p, v)
        return (lambda x, *d: x.transpose(*d))(o, 0, 2, 1, 3).reshape(B, Sq, Hq * Dh) @ wo

    def _B_ref(x, w_r, w_gate, w_up, w_down):
        B, S, D = x.shape
        C = 1
        r = x @ w_r
        idx = jnp.argsort(-r, axis=-1)[:, :C]
        idx_e = jnp.repeat(idx.reshape(B, C, 1), D, axis=2)
        x_sel = jnp.take_along_axis(x, idx_e, axis=1)
        g = _silu(x_sel @ w_gate)
        u = x_sel @ w_up
        y = g * u @ w_down
        r_sel = _sigmoid(jnp.take_along_axis(r, idx, axis=1))
        y = y * r_sel.reshape(B, C, 1)
        b_off = (jnp.arange(B) * S).reshape(B, 1)
        flat_idx = (idx + b_off).reshape(B * C)
        zero = (x * 0.0).reshape(B * S, D)
        upd = _scatter_add(zero, flat_idx, y.reshape(B * C, D), axis=0)
        return x + upd.reshape(B, S, D)
    x = A_x
    mod = (_silu(c) @ w_mod).reshape(c.shape[0], 6, 1, -1)
    sa, ca, ga, sb, cb, gb = (mod[:, 0].copy(), mod[:, 1].copy(), mod[:, 2].copy(), mod[:, 3].copy(), mod[:, 4].copy(), mod[:, 5].copy())
    h = _layernorm(x, axis=-1) * (1 + ca) + sa
    x = x + ga * _A_ref(h, A_k_cache, A_v_cache, A_wq, A_wo)
    h = _layernorm(x, axis=-1) * (1 + cb) + sb
    x = x + gb * _B_ref(h, B_w_r, B_w_gate, B_w_up, B_w_down)
    return x
```

```python
import jax
import jax.numpy as jnp
import jax.experimental.pallas as pl
import jax.experimental.pallas.tpu as pltpu

B, D = 8, 576
HQ, HKV, DH = 32, 16, 128
F = 4608
EPS = 1e-05
NT = (((1,), (1,)), ((), ()))
f32 = jnp.float32
bf16 = jnp.bfloat16


def _layernorm(x):
    m = jnp.mean(x, axis=-1, keepdims=True)
    xc = x - m
    v = jnp.mean(xc * xc, axis=-1, keepdims=True)
    return xc / jnp.sqrt(v + EPS)


def build(DEPTH=5, ROWS=128, LAG_WO=20, LAG_GU=20, bounds=False):

    def kernel(x_hbm, k_hbm, v_hbm, wq_hbm, wo_hbm, wr_hbm, wg_hbm, wu_hbm, wd_hbm, c_hbm, wm_hbm,
               out_ref,
               x_buf, c_buf, wr_buf, wm_buf, wq_buf, wo_buf, wg_buf, wu_buf, wd_buf,
               kbuf, vbuf, q_all, o_all, sem_s, sem_w, sem_d, sem_k, sem_v):
        SK = k_hbm.shape[2]
        W = kbuf.shape[1]
        NG = B * HKV
        scale = DH ** -0.5

        def issue_rows(srcA, dstA, semA, rA, srcB, dstB, semB, rB):
            n = srcA.shape[1]
            half = ((n // 128 + 1) // 2) * 128
            for (c0, cn) in ((0, half), (half, n - half)):
                pltpu.make_async_copy(srcA.at[pl.ds(rA, 8), pl.ds(c0, cn)], dstA.at[pl.ds(rA, 8), pl.ds(c0, cn)],
                                      semA).start(priority=0)
                pltpu.make_async_copy(srcB.at[pl.ds(rB, 8), pl.ds(c0, cn)], dstB.at[pl.ds(rB, 8), pl.ds(c0, cn)],
                                      semB).start(priority=1)

        def issue_split(src, dst, sem, lo, hi):
            def body(t, c):
                r = pl.multiple_of(t * 8, 8)
                issue_rows(src, dst, sem, r, src, dst, sem, pl.multiple_of(r + D // 2, 8))
                return c
            jax.lax.fori_loop(lo, hi, body, 0)

        def issue_pair(srcA, dstA, semA, srcB, dstB, semB, lo, hi):
            def body(t, c):
                r = pl.multiple_of(t * 8, 8)
                issue_rows(srcA, dstA, semA, r, srcB, dstB, semB, r)
                return c
            jax.lax.fori_loop(lo, hi, body, 0)

        def issue_kv(g, slot):
            h = g // B
            b = g % B
            for c in range(W // ROWS):
                pltpu.make_async_copy(k_hbm.at[b, h, pl.ds(SK - W + c * ROWS, ROWS), :],
                                      kbuf.at[slot, pl.ds(c * ROWS, ROWS), :], sem_k.at[slot]).start(priority=0)
                pltpu.make_async_copy(v_hbm.at[b, h, pl.ds(SK - W + c * ROWS, ROWS), :],
                                      vbuf.at[slot, pl.ds(c * ROWS, ROWS), :], sem_v.at[slot]).start(priority=1)

        def wait_all(buf, sem):
            pltpu.make_async_copy(buf, buf, sem).wait()

        cp_c = pltpu.make_async_copy(c_hbm, c_buf, sem_s.at[0])
        cp_x = pltpu.make_async_copy(x_hbm, x_buf, sem_s.at[1])
        cp_r = pltpu.make_async_copy(wr_hbm, wr_buf, sem_s.at[2])
        cp_c.start()
        cp_x.start()
        cp_r.start()
        issue_split(wm_hbm, wm_buf, sem_w.at[0], 0, D // 16)
        issue_split(wq_hbm, wq_buf, sem_w.at[1], 0, D // 16)

        cp_c.wait()
        cp_x.wait()
        cp_r.wait()
        wait_all(wm_buf, sem_w.at[0])
        c = c_buf[...].astype(f32)
        sc = (c * jax.nn.sigmoid(c)).astype(bf16)
        mod = jnp.dot(sc, wm_buf[...], preferred_element_type=f32)
        x0 = x_buf[...].astype(f32)
        sa, ca, ga, sb, cb, gb = [mod[:, i * D:(i + 1) * D] for i in range(6)]
        h1 = (_layernorm(x0) * (1.0 + ca) + sa).astype(bf16)

        def pre(g, c_):
            issue_kv(g, g)
            return c_
        jax.lax.fori_loop(0, DEPTH - 1, pre, 0)

        wait_all(wq_buf, sem_w.at[1])
        q = jnp.dot(h1, wq_buf[...], preferred_element_type=f32)
        for h in range(HKV):
            qh = jnp.concatenate([q[:, (2 * h) * DH:(2 * h + 1) * DH],
                                  q[:, (2 * h + 1) * DH:(2 * h + 2) * DH]], axis=0)
            q_all[h] = qh.astype(bf16)

        row_b = jax.lax.broadcasted_iota(jnp.int32, (2 * B, DH), 0) % B

        def attend(g, o_acc):
            slot = g % DEPTH
            h = g // B
            b = g % B
            wait_all(kbuf.at[slot], sem_k.at[slot])
            s = jax.lax.dot_general(q_all[h], kbuf[slot], NT, preferred_element_type=f32)
            m = jnp.max(s, axis=-1, keepdims=True)
            p = jnp.exp((s - m) * scale)
            l = jnp.sum(p, axis=-1, keepdims=True)
            wait_all(vbuf.at[slot], sem_v.at[slot])
            o = jnp.dot(p.astype(bf16), vbuf[slot], preferred_element_type=f32) / l
            o_acc = jnp.where(row_b == b, o, o_acc)
            o_all[h] = o_acc
            return o_acc

        def main(g, o_acc):
            issue_kv(g + DEPTH - 1, (g + DEPTH - 1) % DEPTH)
            return attend(g, o_acc)

        o_acc = jax.lax.fori_loop(0, NG - (DEPTH - 1), main, jnp.zeros((2 * B, DH), f32))

        NP = D // 16
        per = NP // (DEPTH - 1)

        def tail(i, o_acc):
            issue_split(wo_hbm, wo_buf, sem_w.at[2], i * per, (i + 1) * per)
            return attend(NG - (DEPTH - 1) + i, o_acc)

        o_acc = jax.lax.fori_loop(0, DEPTH - 1, tail, o_acc)
        if per * (DEPTH - 1) < NP:
            issue_split(wo_hbm, wo_buf, sem_w.at[2], per * (DEPTH - 1), NP)

        issue_pair(wg_hbm, wg_buf, sem_w.at[3], wu_hbm, wu_buf, sem_w.at[4], 0, LAG_WO)
        wait_all(wo_buf, sem_w.at[2])
        pieces = []
        for h in range(HKV):
            oh = o_all[h]
            pieces += [oh[:B], oh[B:]]
        o_cat = jnp.concatenate(pieces, axis=1).astype(bf16)
        attn = jax.lax.dot_general(o_cat, wo_buf[...], NT, preferred_element_type=f32)
        x1 = x0 + ga * attn
        h2 = _layernorm(x1) * (1.0 + cb) + sb
        h2b = h2.astype(bf16)
        wr = wr_buf[...].astype(f32).reshape(1, D)
        r = jnp.sum(h2 * wr, axis=-1, keepdims=True)
        rs = jax.nn.sigmoid(r)

        issue_pair(wg_hbm, wg_buf, sem_w.at[3], wu_hbm, wu_buf, sem_w.at[4], LAG_WO, D // 8)

        chunks = [(0, 128), (128, 128), (256, 128), (384, 128), (512, 64)]

        def issue_down(j):
            r0, n = chunks[j]

            def body(t, c_):
                r = pl.multiple_of(r0 + t * 8, 8)
                issue_rows(wd_hbm, wd_buf, sem_d.at[j], r, wd_hbm, wd_buf, sem_d.at[j],
                           pl.multiple_of(r + n // 2, 8))
                return c_
            jax.lax.fori_loop(0, n // 16, body, 0)

        issue_down(0)
        issue_down(1)
        issue_down(2)
        wait_all(wg_buf, sem_w.at[3])
        g_ = jnp.dot(h2b, wg_buf[...], preferred_element_type=f32)
        wait_all(wu_buf, sem_w.at[4])
        u_ = jnp.dot(h2b, wu_buf[...], preferred_element_type=f32)
        act = (g_ * jax.nn.sigmoid(g_) * u_).astype(bf16)
        issue_down(3)
        issue_down(4)
        ys = []
        for j, (r0, n) in enumerate(chunks):
            wait_all(wd_buf.at[pl.ds(r0, n), :], sem_d.at[j])
            ys.append(jax.lax.dot_general(act, wd_buf[pl.ds(r0, n), :], NT, preferred_element_type=f32))
        y = jnp.concatenate(ys, axis=1)
        out = x1 + gb * (h2 + y * rs)
        out_ref[...] = out.astype(out_ref.dtype)

    @jax.jit
    def fn(A_x, A_k_cache, A_v_cache, A_wq, A_wo, B_x, B_w_r, B_w_gate, B_w_up, B_w_down, c, w_mod):
        SK = A_k_cache.shape[2]
        W = min(4096, max(256, SK // 4))
        any_spec = pl.BlockSpec(memory_space=pl.ANY)
        out = pl.pallas_call(
            kernel,
            out_shape=jax.ShapeDtypeStruct((B, D), bf16),
            in_specs=[any_spec] * 11,
            out_specs=pl.BlockSpec(memory_space=pltpu.VMEM),
            scratch_shapes=[
                pltpu.VMEM((B, D), bf16), pltpu.VMEM((B, D), bf16), pltpu.VMEM((D,), bf16),
                pltpu.VMEM((D, 6 * D), bf16), pltpu.VMEM((D, HQ * DH), bf16), pltpu.VMEM((D, HQ * DH), bf16),
                pltpu.VMEM((D, F), bf16), pltpu.VMEM((D, F), bf16), pltpu.VMEM((D, F), bf16),
                pltpu.VMEM((DEPTH, W, DH), bf16), pltpu.VMEM((DEPTH, W, DH), bf16),
                pltpu.VMEM((HKV, 2 * B, DH), bf16), pltpu.VMEM((HKV, 2 * B, DH), f32),
                pltpu.SemaphoreType.DMA((3,)), pltpu.SemaphoreType.DMA((5,)), pltpu.SemaphoreType.DMA((5,)),
                pltpu.SemaphoreType.DMA((DEPTH,)), pltpu.SemaphoreType.DMA((DEPTH,)),
            ],
            compiler_params=pltpu.CompilerParams(vmem_limit_bytes=64 * 1024 * 1024,
                                                 disable_bounds_checks=not bounds),
        )(A_x.reshape(B, D), A_k_cache, A_v_cache, A_wq, A_wo.T, B_w_r, B_w_gate, B_w_up, B_w_down.T, c, w_mod)
        return out.reshape(B, 1, D)

    return fn


pallas_adaLN_cond__sliding_block_cached__moe_arch_mod__decode_kernel = build()
```

```python
import jax
import jax.numpy as jnp
import jax.experimental.pallas as pl
import jax.experimental.pallas.tpu as pltpu

B, D = 8, 576
HQ, HKV, DH = 32, 16, 128
F = 4608
EPS = 1e-05
NT = (((1,), (1,)), ((), ()))
f32 = jnp.float32
bf16 = jnp.bfloat16


def _layernorm(x):
    m = jnp.mean(x, axis=-1, keepdims=True)
    xc = x - m
    v = jnp.mean(xc * xc, axis=-1, keepdims=True)
    return xc / jnp.sqrt(v + EPS)


def build(DEPTH=4, HG=8, CH=256, R=16, NSW=8, LAG_WO=3, check=False):

    def kernel(x_hbm, k_hbm, v_hbm, wq_hbm, wo_hbm, wr_hbm, wg_hbm, wu_hbm, wd_hbm, c_hbm, wm_hbm,
               out_ref,
               x_buf, c_buf, wr_buf, wm_buf, wq_buf, wo_buf, wg_buf, wu_buf, wd_buf,
               kbuf, vbuf, q_all, o_all, sem_s, sem_w, sem_d, sem_k, sem_v):
        SK = k_hbm.shape[2]
        W = min(4096, max(256, SK // 4))
        NC = W // CH
        NS = B * HKV // HG
        NSTEP = NS * NC
        HPB = HKV // HG
        scale = DH ** -0.5

        def halves(n):
            half = ((n // 128 + 1) // 2) * 128
            return ((0, half), (half, n - half))

        def cp(src, dst, sem, r, c0, cn):
            return pltpu.make_async_copy(src.at[pl.ds(r, 8), pl.ds(c0, cn)], dst.at[pl.ds(r, 8), pl.ds(c0, cn)], sem)

        def issue_w(A, Bm, lo, hi):
            def body(t, c_):
                r = t * 8
                for hf in range(2):
                    for s in range(A[4]):
                        for th, M in enumerate((A, Bm)):
                            c0, cn = halves(M[0].shape[1])[hf]
                            cp(M[0], M[1], M[2], pl.multiple_of(M[3] + s * M[5] + r, 8), c0, cn).start(priority=th)
                return c_
            jax.lax.fori_loop(lo, hi, body, 0)

        def whole(src, dst, sem):
            return (src, dst, sem, 0, NSW, D // NSW)

        def split(src, dst, sem, r0=0, n=D, ns=NSW // 2):
            return ((src, dst, sem, r0, ns, n // (2 * ns)), (src, dst, sem, r0 + n // 2, ns, n // (2 * ns)))

        def issue_kv(i, slot):
            t = i // NC
            b = t // HPB
            h0 = (t % HPB) * HG
            r0 = SK - W + (i % NC) * CH
            for c in range(CH // R):
                rr = pl.multiple_of(r0 + c * R, 8)
                pltpu.make_async_copy(k_hbm.at[b, pl.ds(h0, HG), pl.ds(rr, R), :],
                                      kbuf.at[slot, :, pl.ds(c * R, R), :], sem_k.at[slot]).start(priority=0)
                pltpu.make_async_copy(v_hbm.at[b, pl.ds(h0, HG), pl.ds(rr, R), :],
                                      vbuf.at[slot, :, pl.ds(c * R, R), :], sem_v.at[slot]).start(priority=1)

        def wait_all(buf, sem):
            pltpu.make_async_copy(buf, buf, sem).wait()

        cp_c = pltpu.make_async_copy(c_hbm, c_buf, sem_s.at[0])
        cp_x = pltpu.make_async_copy(x_hbm, x_buf, sem_s.at[1])
        cp_r = pltpu.make_async_copy(wr_hbm, wr_buf, sem_s.at[2])
        cp_c.start()
        cp_x.start()
        cp_r.start()
        issue_w(whole(wm_hbm, wm_buf, sem_w.at[0]), whole(wq_hbm, wq_buf, sem_w.at[1]), 0, D // NSW // 8)
        issue_kv(0, 0)

        cp_c.wait()
        cp_x.wait()
        cp_r.wait()
        wait_all(wm_buf, sem_w.at[0])
        c = c_buf[...].astype(f32)
        sc = (c * jax.nn.sigmoid(c)).astype(bf16)
        mod = jnp.dot(sc, wm_buf[...], preferred_element_type=f32)
        x0 = x_buf[...].astype(f32)
        sa, ca, ga, sb, cb, gb = [mod[:, i * D:(i + 1) * D] for i in range(6)]
        h1 = (_layernorm(x0) * (1.0 + ca) + sa).astype(bf16)

        def pre(i, c_):
            issue_kv(i, i)
            return c_
        jax.lax.fori_loop(1, DEPTH - 1, pre, 0)

        wait_all(wq_buf, sem_w.at[1])
        q = jnp.dot(h1, wq_buf[...], preferred_element_type=f32)
        for hq in range(HQ):
            q_all[:, hq, :] = q[:, hq * DH:(hq + 1) * DH]

        QR = 2 * HG
        row_s = jax.lax.broadcasted_iota(jnp.int32, (QR, CH), 0) // 2
        row_o = jax.lax.broadcasted_iota(jnp.int32, (QR, DH), 0) // 2

        def attend(i, qh, m, l, acc):
            slot = i % DEPTH
            wait_all(kbuf.at[slot], sem_k.at[slot])
            s = jax.lax.dot_general(qh, kbuf[slot, 0], NT, preferred_element_type=f32)
            for j in range(1, HG):
                sj = jax.lax.dot_general(qh, kbuf[slot, j], NT, preferred_element_type=f32)
                s = jnp.where(row_s == j, sj, s)
            m_new = jnp.maximum(m, jnp.max(s, axis=-1, keepdims=True))
            alpha = jnp.exp((m - m_new) * scale)
            p = jnp.exp((s - m_new) * scale)
            l = l * alpha + jnp.sum(p, axis=-1, keepdims=True)
            pb = p.astype(bf16)
            wait_all(vbuf.at[slot], sem_v.at[slot])
            o = jnp.dot(pb, vbuf[slot, 0], preferred_element_type=f32)
            for j in range(1, HG):
                oj = jnp.dot(pb, vbuf[slot, j], preferred_element_type=f32)
                o = jnp.where(row_o == j, oj, o)
            return m_new, l, acc * alpha + o

        NWO = D // (NSW // 2) // 2 // 8
        wo_a, wo_b = split(wo_hbm, wo_buf, sem_w.at[2])
        per = -(-NWO // (DEPTH - 1))

        def superstep(t, c_):
            b = t // HPB
            q0 = pl.multiple_of((t % HPB) * QR, QR)
            qh = q_all[b, pl.ds(q0, QR), :].astype(bf16)

            def step(c, carry):
                i = t * NC + c
                nxt = i + DEPTH - 1

                @pl.when(nxt < NSTEP)
                def _():
                    issue_kv(nxt, nxt % DEPTH)

                @pl.when(nxt >= NSTEP)
                def _():
                    e = nxt - NSTEP
                    issue_w(wo_a, wo_b, e * per, jnp.minimum((e + 1) * per, NWO))

                return attend(i, qh, *carry)

            m, l, acc = jax.lax.fori_loop(
                0, NC, step,
                (jnp.full((QR, 1), -jnp.inf, f32), jnp.zeros((QR, 1), f32), jnp.zeros((QR, DH), f32)))
            o_all[b, pl.ds(q0, QR), :] = acc / l
            return c_

        jax.lax.fori_loop(0, NS, superstep, 0)

        wg_s, wu_s = whole(wg_hbm, wg_buf, sem_w.at[3]), whole(wu_hbm, wu_buf, sem_w.at[4])
        NGU = D // NSW // 8
        issue_w(wg_s, wu_s, 0, LAG_WO)
        wait_all(wo_buf, sem_w.at[2])
        o_cat = jnp.concatenate([o_all[:, hq, :] for hq in range(HQ)], axis=1).astype(bf16)
        attn = jax.lax.dot_general(o_cat, wo_buf[...], NT, preferred_element_type=f32)
        x1 = x0 + ga * attn
        h2 = _layernorm(x1) * (1.0 + cb) + sb
        h2b = h2.astype(bf16)
        wr = wr_buf[...].astype(f32).reshape(1, D)
        r = jnp.sum(h2 * wr, axis=-1, keepdims=True)
        rs = jax.nn.sigmoid(r)

        issue_w(wg_s, wu_s, LAG_WO, NGU)

        chunks = [(0, 256, 4), (256, 256, 4), (512, 64, 4)]

        def issue_down(j):
            r0, n, ns = chunks[j]
            a, b_ = split(wd_hbm, wd_buf, sem_d.at[j], r0, n, ns)
            issue_w(a, b_, 0, n // (2 * ns) // 8)

        issue_down(0)
        wait_all(wg_buf, sem_w.at[3])
        g_ = jnp.dot(h2b, wg_buf[...], preferred_element_type=f32)
        g_ = g_ * jax.nn.sigmoid(g_)
        issue_down(1)
        wait_all(wu_buf, sem_w.at[4])
        u_ = jnp.dot(h2b, wu_buf[...], preferred_element_type=f32)
        act = (g_ * u_).astype(bf16)
        issue_down(2)
        ys = []
        for j, (r0, n, _) in enumerate(chunks):
            wait_all(wd_buf.at[pl.ds(r0, n), :], sem_d.at[j])
            ys.append(jax.lax.dot_general(act, wd_buf[pl.ds(r0, n), :], NT, preferred_element_type=f32))
        y = jnp.concatenate(ys, axis=1)
        out = x1 + gb * (h2 + y * rs)
        out_ref[...] = out.astype(out_ref.dtype)

    @jax.jit
    def fn(A_x, A_k_cache, A_v_cache, A_wq, A_wo, B_x, B_w_r, B_w_gate, B_w_up, B_w_down, c, w_mod):
        any_spec = pl.BlockSpec(memory_space=pl.ANY)
        out = pl.pallas_call(
            kernel,
            out_shape=jax.ShapeDtypeStruct((B, D), bf16),
            in_specs=[any_spec] * 11,
            out_specs=pl.BlockSpec(memory_space=pltpu.VMEM),
            scratch_shapes=[
                pltpu.VMEM((B, D), bf16), pltpu.VMEM((B, D), bf16), pltpu.VMEM((D,), bf16),
                pltpu.VMEM((D, 6 * D), bf16), pltpu.VMEM((D, HQ * DH), bf16), pltpu.VMEM((D, HQ * DH), bf16),
                pltpu.VMEM((D, F), bf16), pltpu.VMEM((D, F), bf16), pltpu.VMEM((D, F), bf16),
                pltpu.VMEM((DEPTH, HG, CH, DH), bf16), pltpu.VMEM((DEPTH, HG, CH, DH), bf16),
                pltpu.VMEM((B, HQ, DH), f32), pltpu.VMEM((B, HQ, DH), f32),
                pltpu.SemaphoreType.DMA((3,)), pltpu.SemaphoreType.DMA((5,)), pltpu.SemaphoreType.DMA((5,)),
                pltpu.SemaphoreType.DMA((DEPTH,)), pltpu.SemaphoreType.DMA((DEPTH,)),
            ],
            compiler_params=pltpu.CompilerParams(vmem_limit_bytes=64 * 1024 * 1024,
                                                 disable_bounds_checks=not check,
                                                 disable_semaphore_checks=not check),
        )(A_x.reshape(B, D), A_k_cache, A_v_cache, A_wq, A_wo.T, B_w_r, B_w_gate, B_w_up, B_w_down.T, c, w_mod)
        return out.reshape(B, 1, D)

    return fn


pallas_adaLN_cond__sliding_block_cached__moe_arch_mod__decode_kernel = build()
```

```python
import jax
import jax.numpy as jnp
import jax.experimental.pallas as pl
import jax.experimental.pallas.tpu as pltpu

B, D = 8, 576
HQ, HKV, DH = 32, 16, 128
F = 4608
EPS = 1e-05
NT = (((1,), (1,)), ((), ()))
f32 = jnp.float32
bf16 = jnp.bfloat16


def _layernorm(x):
    m = jnp.mean(x, axis=-1, keepdims=True)
    xc = x - m
    v = jnp.mean(xc * xc, axis=-1, keepdims=True)
    return xc / jnp.sqrt(v + EPS)


def _pieces(blk0, nblk, rows, ncols, cw, c_lo=0):
    return [(blk0, nblk, r, c0, min(cw, ncols - c0)) for r in range(0, rows, 8) for c0 in range(c_lo, ncols, cw)]


def build(DEPTH=4, HG=8, CH=256, R=16, LAG=26, P_WO=0, P_G=70, P_U=30, CSPLIT=2304,
          NB_M=4, CW_M=640, NB_Q=9, CW_Q=256, NB_G=6, CW_G=384, check=False, skip=(), prof=False):
    NPAD = LAG
    import contextlib
    scope = jax.named_scope if prof else (lambda n: contextlib.nullcontext())
    NB_D = 9
    RD = D // NB_D

    def kernel(x_hbm, k_hbm, v_hbm, wq_hbm, wo_hbm, wr_hbm, wg_hbm, wu_hbm, wd_hbm, c_hbm, wm_hbm,
               out_ref,
               x_buf, c_buf, wr_buf, wm_buf, wq_buf, wo_buf, wg_buf, wu_buf, wd_buf, pad_buf,
               kbuf, vbuf, q_all, o_all, fin, flag, sems):
        SK = k_hbm.shape[2]
        W = min(4096, max(256, SK // 4))
        NC = W // CH
        NS = B * HKV // HG
        NSTEP = NS * NC
        HPB = HKV // HG
        scale = DH ** -0.5

        class _Sub:
            def __init__(self, off):
                self.off = off
                self.at = self

            def __getitem__(self, i):
                return sems.at[self.off + i]

        sem_s, sem_w, sem_d, sem_k, sem_v = _Sub(0), _Sub(4), _Sub(9), _Sub(13), _Sub(13 + DEPTH)
        flag[0] = 1

        def wcopy(src, dst, sem, p):
            b0, nb, r, c0, cn = p
            idx = (pl.ds(b0, nb), pl.ds(r, 8), pl.ds(c0, cn))
            return pltpu.make_async_copy(src.at[idx], dst.at[idx], sem)

        def issue_kv(i, slot):
            t = i // NC
            b = t // HPB
            h0 = (t % HPB) * HG
            r0 = SK - W + (i % NC) * CH
            for c in range(CH // R):
                rr = pl.multiple_of(r0 + c * R, 8)
                pltpu.make_async_copy(k_hbm.at[b, pl.ds(h0, HG), pl.ds(rr, R), :],
                                      kbuf.at[slot, :, pl.ds(c * R, R), :], sem_k.at[slot]).start(priority=0)
                pltpu.make_async_copy(v_hbm.at[b, pl.ds(h0, HG), pl.ds(rr, R), :],
                                      vbuf.at[slot, :, pl.ds(c * R, R), :], sem_v.at[slot]).start(priority=1)

        def wait_all(buf, sem):
            pltpu.make_async_copy(buf, buf, sem).wait()

        s0 = [wcopy(wm_hbm, wm_buf, sem_w.at[0], p) for p in _pieces(0, NB_M, D // NB_M, 6 * D, CW_M)]
        s1 = [wcopy(wq_hbm, wq_buf, sem_w.at[1], p) for p in _pieces(0, NB_Q, D // NB_Q, HQ * DH, CW_Q)]
        lead = len(s1) - len(s0)
        assert lead >= 0
        cp_c = pltpu.make_async_copy(c_hbm, c_buf, sem_s.at[0])
        cp_x = pltpu.make_async_copy(x_hbm, x_buf, sem_s.at[1])
        cp_r = pltpu.make_async_copy(wr_hbm, wr_buf, sem_s.at[2])
        for d in s1[:lead]:
            d.start(priority=1)
        cp_c.start()
        cp_x.start()
        cp_r.start()
        for d0, d1 in zip(s0, s1[lead:]):
            d0.start(priority=0)
            d1.start(priority=1)

        def pre(i, c_):
            issue_kv(i, i)
            return c_
        jax.lax.fori_loop(0, 2, pre, 0)

        cp_c.wait()
        cp_x.wait()
        cp_r.wait()
        wait_all(wm_buf, sem_w.at[0])
        c = c_buf[...].astype(f32)
        sc = (c * jax.nn.sigmoid(c)).astype(bf16)
        mod = wm_buf[0, 0:8, :].astype(f32) if 'mod' in skip else jnp.dot(sc, wm_buf[...].reshape(D, 6 * D), preferred_element_type=f32)
        x0 = x_buf[...].astype(f32)
        sa, ca, ga, sb, cb, gb = [mod[:, i * D:(i + 1) * D] for i in range(6)]
        h1 = (_layernorm(x0) * (1.0 + ca) + sa).astype(bf16)

        jax.lax.fori_loop(2, DEPTH - 1, pre, 0)

        wait_all(wq_buf, sem_w.at[1])
        q = (wq_buf[0, 0:8, :].astype(f32) + h1[:, 0:1].astype(f32)) if 'q' in skip else jnp.dot(h1, wq_buf[...].reshape(D, HQ * DH), preferred_element_type=f32)
        for hq in range(HQ):
            q_all[:, hq, :] = q[:, hq * DH:(hq + 1) * DH]

        NWO_LOOP = D // 8 - LAG // 2
        HW = HQ * DH // 2

        def wo_copy(r, th):
            idx = (pl.ds(r, 8), pl.ds(th * HW, HW))
            return pltpu.make_async_copy(wo_hbm.at[idx], wo_buf.at[idx], sem_w.at[2])

        e0 = [wo_copy(8 * t, th) for t in range(NWO_LOOP, D // 8) for th in range(2)]
        e0 += [wcopy(wg_hbm, wg_buf, sem_w.at[3], p) for p in _pieces(0, NB_G, D // NB_G, F, CW_G)]
        e1 = [wcopy(wu_hbm, wu_buf, sem_w.at[4], p) for p in _pieces(0, NB_G, D // NB_G, F, CW_G)]
        n_g = len(e0)
        e0 += [wcopy(wd_hbm, wd_buf, sem_d.at[0], p) for p in _pieces(0, 3, RD, F, 768)]
        e1 += [wcopy(wd_hbm, wd_buf, sem_d.at[0], p) for p in _pieces(3, 3, RD, F, 768)]
        e0 += [wcopy(wd_hbm, wd_buf, sem_d.at[1], p) for p in _pieces(6, 1, RD, F, F // 2)]
        e1 += [wcopy(wd_hbm, wd_buf, sem_d.at[1], p) for p in _pieces(7, 1, RD, F, F // 2)]
        c1 = [wcopy(wd_hbm, wd_buf, sem_d.at[2], p) for p in _pieces(8, 1, RD, CSPLIT, CSPLIT)]
        c2 = [wcopy(wd_hbm, wd_buf, sem_d.at[3], p) for p in _pieces(8, 1, RD, F, F - CSPLIT, CSPLIT)]
        e0 += c1[:4] + c2[:4]
        e1 += c1[4:] + c2[4:]
        npad = len(e0) - len(e1)
        e1 += [pltpu.make_async_copy(wo_hbm.at[pl.ds(0, 8), pl.ds(128 * j, 128)], pad_buf.at[j], sem_s.at[3])
               for j in range(npad)]
        eseq = []
        for i0, (d0, d1) in enumerate(zip(e0, e1)):
            eseq += [(d0, 0, i0), (d1, 1, i0)]
        epos = [0]

        def issue_end(upto):
            upto = min(upto, len(eseq))
            todo = eseq[epos[0]:upto]
            epos[0] = max(epos[0], upto)
            if todo:
                @pl.when(flag[0] == 1)
                def _():
                    for d, th, _i in todo:
                        d.start(priority=th)

        def pos_after(th, idx):
            return next(n for n, (_, t_, i_) in enumerate(eseq) if t_ == th and i_ == idx) + 1

        QR = 2 * HG
        row_s = jax.lax.broadcasted_iota(jnp.int32, (QR, CH), 0) // 2
        row_o = jax.lax.broadcasted_iota(jnp.int32, (QR, DH), 0) // 2

        def attend(i, qh, m, l, acc):
            slot = i % DEPTH
            wait_all(kbuf.at[slot], sem_k.at[slot])
            if 'attn' in skip:
                wait_all(vbuf.at[slot], sem_v.at[slot])
                return m, l + 1.0, acc + kbuf[slot, 0, 0:16, :].astype(f32) + vbuf[slot, 0, 0:16, :].astype(f32)
            s = jax.lax.dot_general(qh, kbuf[slot, 0], NT, preferred_element_type=f32)
            for j in range(1, HG):
                sj = jax.lax.dot_general(qh, kbuf[slot, j], NT, preferred_element_type=f32)
                s = jnp.where(row_s == j, sj, s)
            m_new = jnp.maximum(m, jnp.max(s, axis=-1, keepdims=True))
            alpha = jnp.exp((m - m_new) * scale)
            p = jnp.exp((s - m_new) * scale)
            l = l * alpha + jnp.sum(p, axis=-1, keepdims=True)
            pb = p.astype(bf16)
            wait_all(vbuf.at[slot], sem_v.at[slot])
            o = jnp.dot(pb, vbuf[slot, 0], preferred_element_type=f32)
            for j in range(1, HG):
                oj = jnp.dot(pb, vbuf[slot, j], preferred_element_type=f32)
                o = jnp.where(row_o == j, oj, o)
            return m_new, l, acc * alpha + o

        PER = 2 * (CH // R)
        tail_issue = []
        for e in range(DEPTH - 1):
            tail_issue.append(eseq[e * PER:(e + 1) * PER])
        epos[0] = (DEPTH - 1) * PER

        def superstep(t, c_):
            b = t // HPB
            q0 = pl.multiple_of((t % HPB) * QR, QR)
            qh = q_all[b, pl.ds(q0, QR), :].astype(bf16)

            def step(c, carry):
                i = t * NC + c
                nxt = i + DEPTH - 1

                @pl.when(nxt < NSTEP)
                def _():
                    issue_kv(nxt, nxt % DEPTH)

                @pl.when(i < NWO_LOOP)
                def _():
                    r = pl.multiple_of(i * 8, 8)
                    for th in range(2):
                        wo_copy(r, th).start(priority=th)

                for e in range(DEPTH - 1):
                    @pl.when(nxt == NSTEP + e)
                    def _():
                        for d, th, _i in tail_issue[e]:
                            d.start(priority=th)

                return attend(i, qh, *carry)

            m, l, acc = jax.lax.fori_loop(
                0, NC, step,
                (jnp.full((QR, 1), -jnp.inf, f32), jnp.zeros((QR, 1), f32), jnp.zeros((QR, DH), f32)))
            o_all[b, pl.ds(q0, QR), :] = acc / l
            return c_

        jax.lax.fori_loop(0, NS, superstep, 0)

        issue_end(epos[0] + P_WO)
        with scope("wO"):
            wait_all(wo_buf, sem_w.at[2])
        with scope("cO"):
            o_cat = jnp.concatenate([o_all[:, hq, :] for hq in range(HQ)], axis=1).astype(bf16)
            attn = jax.lax.dot_general(o_cat, wo_buf[...], NT, preferred_element_type=f32)
            x1 = x0 + ga * attn
            h2 = _layernorm(x1) * (1.0 + cb) + sb
            h2b = h2.astype(bf16)
            wr = wr_buf[...].astype(f32).reshape(1, D)
            r = jnp.sum(h2 * wr, axis=-1, keepdims=True)
            fin[0] = x1 + gb * h2
            fin[1] = gb * jax.nn.sigmoid(r)

        with scope("iG"):
            issue_end(pos_after(0, n_g - 1) + P_G)
        with scope("wG"):
            wait_all(wg_buf, sem_w.at[3])
        with scope("cG"):
            g_ = jnp.dot(h2b, wg_buf[...].reshape(D, F), preferred_element_type=f32)
            g_ = g_ * jax.nn.sigmoid(g_)
        with scope("iU"):
            issue_end(epos[0] + P_U)
        with scope("wU"):
            wait_all(wu_buf, sem_w.at[4])
        with scope("cU"):
            u_ = jnp.dot(h2b, wu_buf[...].reshape(D, F), preferred_element_type=f32)
            act = (g_ * u_).astype(bf16)
        with scope("iL"):
            issue_end(len(eseq))

        def down(a, w):
            if 'down' in skip:
                return a[:, :w.shape[0]].astype(f32) + w[0:8, 0:w.shape[0]].astype(f32)
            return jax.lax.dot_general(a, w, NT, preferred_element_type=f32)

        def fin_at(lo, hi, y):
            return fin[0, :, lo:hi] + fin[1, :, lo:hi] * y

        with scope("wA"):
            wait_all(wd_buf.at[pl.ds(0, 6)], sem_d.at[0])
        with scope("cA"):
            ya = down(act, wd_buf[pl.ds(0, 6)].reshape(6 * RD, F))
            out_ref[:, 0:6 * RD] = fin_at(0, 6 * RD, ya).astype(out_ref.dtype)
        with scope("wB"):
            wait_all(wd_buf.at[pl.ds(6, 2)], sem_d.at[1])
        with scope("cB"):
            yb = down(act, wd_buf[pl.ds(6, 2)].reshape(2 * RD, F))
            out_ref[:, 6 * RD:8 * RD] = fin_at(6 * RD, 8 * RD, yb).astype(out_ref.dtype)
        with scope("wC1"):
            wait_all(wd_buf.at[8, :, pl.ds(0, CSPLIT)], sem_d.at[2])
        with scope("cC1"):
            yc = down(act[:, :CSPLIT], wd_buf[8, :, pl.ds(0, CSPLIT)])
            fin[0, :, 8 * RD:] = fin_at(8 * RD, D, yc)
        with scope("wC2"):
            wait_all(wd_buf.at[8, :, pl.ds(CSPLIT, F - CSPLIT)], sem_d.at[3])
        with scope("cC2"):
            yc = down(act[:, CSPLIT:], wd_buf[8, :, pl.ds(CSPLIT, F - CSPLIT)])
            out_ref[:, 8 * RD:] = fin_at(8 * RD, D, yc).astype(out_ref.dtype)
        with scope("wPad"):
            wait_all(pad_buf.at[pl.ds(0, npad)], sem_s.at[3])

    @jax.jit
    def fn(A_x, A_k_cache, A_v_cache, A_wq, A_wo, B_x, B_w_r, B_w_gate, B_w_up, B_w_down, c, w_mod):
        any_spec = pl.BlockSpec(memory_space=pl.ANY)
        out = pl.pallas_call(
            kernel,
            out_shape=jax.ShapeDtypeStruct((B, D), bf16),
            in_specs=[any_spec] * 11,
            out_specs=pl.BlockSpec(memory_space=pltpu.VMEM),
            scratch_shapes=[
                pltpu.VMEM((B, D), bf16), pltpu.VMEM((B, D), bf16), pltpu.VMEM((D,), bf16),
                pltpu.VMEM((NB_M, D // NB_M, 6 * D), bf16), pltpu.VMEM((NB_Q, D // NB_Q, HQ * DH), bf16),
                pltpu.VMEM((D, HQ * DH), bf16),
                pltpu.VMEM((NB_G, D // NB_G, F), bf16), pltpu.VMEM((NB_G, D // NB_G, F), bf16),
                pltpu.VMEM((NB_D, RD, F), bf16), pltpu.VMEM((max(NPAD, 1), B, 128), bf16),
                pltpu.VMEM((DEPTH, HG, CH, DH), bf16), pltpu.VMEM((DEPTH, HG, CH, DH), bf16),
                pltpu.VMEM((B, HQ, DH), f32), pltpu.VMEM((B, HQ, DH), f32), pltpu.VMEM((2, B, D), f32),
                pltpu.SMEM((1,), jnp.int32), pltpu.SemaphoreType.DMA((13 + 2 * DEPTH,)),
            ],
            compiler_params=pltpu.CompilerParams(vmem_limit_bytes=64 * 1024 * 1024,
                                                 disable_bounds_checks=not check,
                                                 disable_semaphore_checks=not check),
        )(A_x.reshape(B, D), A_k_cache, A_v_cache, A_wq.reshape(NB_Q, D // NB_Q, HQ * DH), A_wo.T, B_w_r,
          B_w_gate.reshape(NB_G, D // NB_G, F), B_w_up.reshape(NB_G, D // NB_G, F),
          B_w_down.T.reshape(NB_D, RD, F), c, w_mod.reshape(NB_M, D // NB_M, 6 * D))
        return out.reshape(B, 1, D)

    return fn


pallas_adaLN_cond__sliding_block_cached__moe_arch_mod__decode_kernel = build()
```

```python
import jax
import jax.numpy as jnp
import jax.experimental.pallas as pl
import jax.experimental.pallas.tpu as pltpu

B, D = 8, 576
HQ, HKV, DH = 32, 16, 128
F = 4608
EPS = 1e-05
NT = (((1,), (1,)), ((), ()))
f32 = jnp.float32
bf16 = jnp.bfloat16


def _layernorm(x):
    m = jnp.mean(x, axis=-1, keepdims=True)
    xc = x - m
    v = jnp.mean(xc * xc, axis=-1, keepdims=True)
    return xc / jnp.sqrt(v + EPS)


def _pieces(blk0, nblk, rows, c_lo, c_hi, cw):
    return [(blk0, nblk, r, c0, min(cw, c_hi - c0)) for r in range(0, rows, 8) for c0 in range(c_lo, c_hi, cw)]


def build(DEPTH=4, LAG=26, P_WO=12, P_O2=24, P_G=70, P_U=30, CSPLIT=2816, CW_M=640, CW_A=768, check=False):
    HG, CH, R = 8, 256, 16
    NB_M, NB = 4, 9
    RB = D // NB
    QR = 2 * HG
    HW = HQ * DH // 2
    S_C, S_X, S_R, S_PAD, S_M, S_Q, S_O, S_G, S_U, S_D, S_K = 0, 1, 2, 3, 4, 5, 6, 7, 8, 9, 13
    S_V = S_K + DEPTH
    STAGES = ((0, 6, 0, F), (6, 8, 0, F), (8, 9, 0, CSPLIT), (8, 9, CSPLIT, F))

    def kernel(x_hbm, k_hbm, v_hbm, wq_hbm, wo_hbm, wr_hbm, wg_hbm, wu_hbm, wd_hbm, c_hbm, wm_hbm,
               out_ref,
               x_buf, c_buf, wr_buf, wm_buf, wq_buf, wo_buf, wg_buf, wu_buf, wd_buf, pad_buf,
               kbuf, vbuf, q_all, o_all, fin, flag, sems):
        SK = k_hbm.shape[2]
        W = min(4096, max(256, SK // 4))
        NC = W // CH
        HPB = HKV // HG
        NS = B * HPB
        NSTEP = NS * NC
        scale = DH ** -0.5
        flag[0] = 1

        def wcopies(src, dst, s, ps):
            out = []
            for b0, nb, r, c0, cn in ps:
                idx = (pl.ds(b0, nb), pl.ds(r, 8), pl.ds(c0, cn))
                out.append(pltpu.make_async_copy(src.at[idx], dst.at[idx], sems.at[s]))
            return out

        def wo_copy(r, half):
            idx = (pl.ds(r, 8), pl.ds(half * HW, HW))
            return pltpu.make_async_copy(wo_hbm.at[idx], wo_buf.at[idx], sems.at[S_O])

        def issue_kv(i, slot):
            t = i // NC
            b = t // HPB
            h0 = (t % HPB) * HG
            r0 = SK - W + (i % NC) * CH
            for c in range(CH // R):
                rows = pl.ds(pl.multiple_of(r0 + c * R, R), R)
                pltpu.make_async_copy(k_hbm.at[b, pl.ds(h0, HG), rows, :], kbuf.at[slot, :, pl.ds(c * R, R), :],
                                      sems.at[S_K + slot]).start(priority=0)
                pltpu.make_async_copy(v_hbm.at[b, pl.ds(h0, HG), rows, :], vbuf.at[slot, :, pl.ds(c * R, R), :],
                                      sems.at[S_V + slot]).start(priority=1)

        def wait_all(buf, s):
            pltpu.make_async_copy(buf, buf, sems.at[s]).wait()

        def block(fn):
            pl.when(flag[0] == 1)(fn)

        s0 = wcopies(wm_hbm, wm_buf, S_M, _pieces(0, NB_M, D // NB_M, 0, 6 * D, CW_M))
        s1 = wcopies(wq_hbm, wq_buf, S_Q, _pieces(0, NB, RB, 0, HQ * DH, 256))
        lead = len(s1) - len(s0)
        small = [pltpu.make_async_copy(c_hbm, c_buf, sems.at[S_C]),
                 pltpu.make_async_copy(x_hbm, x_buf, sems.at[S_X]),
                 pltpu.make_async_copy(wr_hbm, wr_buf, sems.at[S_R])]
        for d in s1[:lead] + small:
            d.start(priority=1)
        for d0, d1 in zip(s0, s1[lead:]):
            d0.start(priority=0)
            d1.start(priority=1)

        def pre(i, carry):
            issue_kv(i, i)
            return carry

        jax.lax.fori_loop(0, 2, pre, 0)

        for d in small:
            d.wait()
        wait_all(wm_buf, S_M)
        c = c_buf[...].astype(f32)
        sc = (c * jax.nn.sigmoid(c)).astype(bf16)
        mod = jnp.dot(sc, wm_buf[...].reshape(D, 6 * D), preferred_element_type=f32)
        sa, ca, ga, sb, cb, gb = [mod[:, i * D:(i + 1) * D] for i in range(6)]
        x0 = x_buf[...].astype(f32)
        h1 = (_layernorm(x0) * (1.0 + ca) + sa).astype(bf16)

        block(lambda: issue_kv(2, 2))
        wait_all(wq_buf, S_Q)
        for half in range(2):
            q = jnp.dot(h1, wq_buf[:, :, half * HW:(half + 1) * HW].reshape(D, HW), preferred_element_type=f32)
            for j in range(HQ // 2):
                q_all[:, half * (HQ // 2) + j, :] = q[:, j * DH:(j + 1) * DH]
            if 3 + half < DEPTH - 1:
                block(lambda: issue_kv(3 + half, 3 + half))
        assert DEPTH <= 6

        n_wo_loop = D // 8 - LAG // 2
        gu_pieces = _pieces(0, 8, RB, 0, F, 256) + _pieces(8, 1, RB, 0, F, F // 2)
        e0 = [wo_copy(8 * t, half) for t in range(n_wo_loop, D // 8) for half in range(2)]
        e0 += wcopies(wg_hbm, wg_buf, S_G, gu_pieces)
        e1 = wcopies(wu_hbm, wu_buf, S_U, gu_pieces)
        n_g = len(e0)
        for j, (bl, bh, cl, ch) in enumerate(STAGES):
            nb = (bh - bl) // 2
            if nb:
                cw = CW_A if nb > 1 else F // 2
                e0 += wcopies(wd_hbm, wd_buf, S_D + j, _pieces(bl, nb, RB, cl, ch, cw))
                e1 += wcopies(wd_hbm, wd_buf, S_D + j, _pieces(bl + nb, nb, RB, cl, ch, cw))
            else:
                ps = wcopies(wd_hbm, wd_buf, S_D + j, _pieces(bl, 1, RB, cl, ch, ch - cl))
                e0 += ps[:len(ps) // 2]
                e1 += ps[len(ps) // 2:]
        assert len(e0) - len(e1) == pad_buf.shape[0]
        e1 += [pltpu.make_async_copy(wo_hbm.at[pl.ds(0, 8), pl.ds(128 * j, 128)], pad_buf.at[j], sems.at[S_PAD])
               for j in range(pad_buf.shape[0])]
        eseq = [x for d0, d1 in zip(e0, e1) for x in ((d0, 0), (d1, 1))]

        def issue_range(lo, hi):
            for d, prio in eseq[lo:hi]:
                d.start(priority=prio)

        row_s = jax.lax.broadcasted_iota(jnp.int32, (QR, CH), 0) // 2
        row_o = jax.lax.broadcasted_iota(jnp.int32, (QR, DH), 0) // 2
        per_step = 2 * (CH // R)

        def superstep(t, carry):
            b = t // HPB
            q0 = pl.multiple_of((t % HPB) * QR, QR)
            qh = q_all[b, pl.ds(q0, QR), :].astype(bf16)

            def step(c, state):
                m, l, acc = state
                i = t * NC + c
                slot = i % DEPTH
                nxt = i + DEPTH - 1

                @pl.when(nxt < NSTEP)
                def _():
                    issue_kv(nxt, nxt % DEPTH)

                @pl.when(i < n_wo_loop)
                def _():
                    for half in range(2):
                        wo_copy(pl.multiple_of(i * 8, 8), half).start(priority=half)

                for e in range(DEPTH - 1):
                    @pl.when(nxt == NSTEP + e)
                    def _():
                        issue_range(e * per_step, (e + 1) * per_step)

                wait_all(kbuf.at[slot], S_K + slot)
                s = jax.lax.dot_general(qh, kbuf[slot, 0], NT, preferred_element_type=f32)
                for j in range(1, HG):
                    sj = jax.lax.dot_general(qh, kbuf[slot, j], NT, preferred_element_type=f32)
                    s = jnp.where(row_s == j, sj, s)
                m_new = jnp.maximum(m, jnp.max(s, axis=-1, keepdims=True))
                alpha = jnp.exp((m - m_new) * scale)
                p = jnp.exp((s - m_new) * scale)
                l = l * alpha + jnp.sum(p, axis=-1, keepdims=True)
                pb = p.astype(bf16)
                wait_all(vbuf.at[slot], S_V + slot)
                o = jnp.dot(pb, vbuf[slot, 0], preferred_element_type=f32)
                for j in range(1, HG):
                    oj = jnp.dot(pb, vbuf[slot, j], preferred_element_type=f32)
                    o = jnp.where(row_o == j, oj, o)
                return m_new, l, acc * alpha + o

            init = (jnp.full((QR, 1), -jnp.inf, f32), jnp.zeros((QR, 1), f32), jnp.zeros((QR, DH), f32))
            _, l, acc = jax.lax.fori_loop(0, NC, step, init)
            o_all[b, pl.ds(q0, QR), :] = acc / l
            return carry

        jax.lax.fori_loop(0, NS, superstep, 0)

        p0 = (DEPTH - 1) * per_step
        cuts = [p0, p0 + P_WO, p0 + P_WO + P_O2, 2 * n_g + P_G, 2 * n_g + P_G + P_U, len(eseq)]

        def issue_part(n):
            block(lambda: issue_range(cuts[n], cuts[n + 1]))

        issue_part(0)
        wait_all(wo_buf, S_O)
        attn = None
        for half in range(2):
            o_cat = jnp.concatenate([o_all[:, half * (HQ // 2) + j, :] for j in range(HQ // 2)], axis=1)
            part = jax.lax.dot_general(o_cat.astype(bf16), wo_buf[:, half * HW:(half + 1) * HW], NT,
                                       preferred_element_type=f32)
            if half == 0:
                attn = part
                issue_part(1)
            else:
                attn = attn + part
        x1 = x0 + ga * attn
        h2 = _layernorm(x1) * (1.0 + cb) + sb
        h2b = h2.astype(bf16)
        r = jnp.sum(h2 * wr_buf[...].astype(f32).reshape(1, D), axis=-1, keepdims=True)
        fin[0] = x1 + gb * h2
        fin[1] = gb * jax.nn.sigmoid(r)

        issue_part(2)
        wait_all(wg_buf, S_G)
        g = jnp.dot(h2b, wg_buf[...].reshape(D, F), preferred_element_type=f32)
        g = g * jax.nn.sigmoid(g)
        issue_part(3)
        wait_all(wu_buf, S_U)
        u = jnp.dot(h2b, wu_buf[...].reshape(D, F), preferred_element_type=f32)
        act = (g * u).astype(bf16)
        issue_part(4)

        for j, (bl, bh, cl, ch) in enumerate(STAGES):
            view = (pl.ds(bl, bh - bl), slice(None), pl.ds(cl, ch - cl))
            lo, hi = bl * RB, bh * RB
            wait_all(wd_buf.at[view], S_D + j)
            y = jax.lax.dot_general(act[:, cl:ch], wd_buf[view].reshape(hi - lo, ch - cl), NT,
                                    preferred_element_type=f32)
            res = fin[0, :, lo:hi] + fin[1, :, lo:hi] * y
            if ch == F:
                out_ref[:, lo:hi] = res.astype(out_ref.dtype)
            else:
                fin[0, :, lo:hi] = res
        wait_all(pad_buf, S_PAD)

    @jax.jit
    def fn(A_x, A_k_cache, A_v_cache, A_wq, A_wo, B_x, B_w_r, B_w_gate, B_w_up, B_w_down, c, w_mod):
        out = pl.pallas_call(
            kernel,
            out_shape=jax.ShapeDtypeStruct((B, D), bf16),
            in_specs=[pl.BlockSpec(memory_space=pl.ANY)] * 11,
            out_specs=pl.BlockSpec(memory_space=pltpu.VMEM),
            scratch_shapes=[
                pltpu.VMEM((B, D), bf16), pltpu.VMEM((B, D), bf16), pltpu.VMEM((D,), bf16),
                pltpu.VMEM((NB_M, D // NB_M, 6 * D), bf16), pltpu.VMEM((NB, RB, HQ * DH), bf16),
                pltpu.VMEM((D, HQ * DH), bf16),
                pltpu.VMEM((NB, RB, F), bf16), pltpu.VMEM((NB, RB, F), bf16), pltpu.VMEM((NB, RB, F), bf16),
                pltpu.VMEM((LAG // 2 * 2, 8, 128), bf16),
                pltpu.VMEM((DEPTH, HG, CH, DH), bf16), pltpu.VMEM((DEPTH, HG, CH, DH), bf16),
                pltpu.VMEM((B, HQ, DH), f32), pltpu.VMEM((B, HQ, DH), f32), pltpu.VMEM((2, B, D), f32),
                pltpu.SMEM((1,), jnp.int32), pltpu.SemaphoreType.DMA((S_V + DEPTH,)),
            ],
            compiler_params=pltpu.CompilerParams(vmem_limit_bytes=64 * 1024 * 1024,
                                                 disable_bounds_checks=not check,
                                                 disable_semaphore_checks=not check),
        )(A_x.reshape(B, D), A_k_cache, A_v_cache, A_wq.reshape(NB, RB, HQ * DH), A_wo.T, B_w_r,
          B_w_gate.reshape(NB, RB, F), B_w_up.reshape(NB, RB, F), B_w_down.T.reshape(NB, RB, F),
          c, w_mod.reshape(NB_M, D // NB_M, 6 * D))
        return out.reshape(B, 1, D)

    return fn


pallas_adaLN_cond__sliding_block_cached__moe_arch_mod__decode_kernel = build()
```

```python
import jax
import jax.numpy as jnp
import jax.experimental.pallas as pl
import jax.experimental.pallas.tpu as pltpu

B, D = 8, 576
HQ, HKV, DH = 32, 16, 128
F = 4608
EPS = 1e-05
NT = (((1,), (1,)), ((), ()))
f32 = jnp.float32
bf16 = jnp.bfloat16


def _layernorm(x):
    m = jnp.mean(x, axis=-1, keepdims=True)
    xc = x - m
    v = jnp.mean(xc * xc, axis=-1, keepdims=True)
    return xc / jnp.sqrt(v + EPS)


def _pieces(blk0, nblk, rows, c_lo, c_hi, cw):
    return [(blk0, nblk, r, c0, min(cw, c_hi - c0)) for r in range(0, rows, 8) for c0 in range(c_lo, c_hi, cw)]


def build(DEPTH=4, LAG=26, LV=2, ST=2, GU=((0,5,384),(5,4,512)), QS=((0,1,2048),(1,8,256)), P_WO=12, P_O2=24, P_G=70, P_U=30, CSPLIT=2816, CW_M=512, CW_A=768, check=False):
    HG, CH, R = 8, 256, 16
    NB_M, NB = 4, 9
    RB = D // NB
    QR = 2 * HG
    HW = HQ * DH // 2
    S_C, S_X, S_R, S_PAD, S_M, S_Q, S_O, S_G, S_U, S_D, S_K = 0, 1, 2, 3, 4, 5, 6, 7, 8, 9, 13
    S_V = S_K + DEPTH
    DV = DEPTH + 1
    NPC = CH // R
    STAGES = ((0, 6, 0, F), (6, 8, 0, F), (8, 9, 0, CSPLIT), (8, 9, CSPLIT, F))

    def kernel(x_hbm, k_hbm, v_hbm, wq_hbm, wo_hbm, wr_hbm, wg_hbm, wu_hbm, wd_hbm, c_hbm, wm_hbm,
               out_ref,
               x_buf, c_buf, wr_buf, wm_buf, wq_buf, wo_buf, wg_buf, wu_buf, wd_buf, pad_buf,
               kbuf, vbuf, q_all, o_all, fin, flag, sems):
        SK = k_hbm.shape[3]
        W = min(4096, max(256, SK // 4))
        NC = W // CH
        HPB = HKV // HG
        NS = B * HPB
        NSTEP = NS * NC
        scale = DH ** -0.5
        flag[0] = 1

        def wcopies(src, dst, s, ps):
            out = []
            for b0, nb, r, c0, cn in ps:
                idx = (pl.ds(b0, nb), pl.ds(r, 8), pl.ds(c0, cn))
                out.append(pltpu.make_async_copy(src.at[idx], dst.at[idx], sems.at[s]))
            return out

        def wo_copy(r, half):
            idx = (pl.ds(r, 8), pl.ds(half * HW, HW))
            return pltpu.make_async_copy(wo_hbm.at[idx], wo_buf.at[idx], sems.at[S_O])

        def kv_copy(src, buf, s0, i, c):
            t = i // NC
            rows = pl.ds(pl.multiple_of(SK - W + (i % NC) * CH + c * R, R), R)
            slot = i % buf.shape[0]
            if ST == 2:
                ref = src.at[t // HPB, :, t % HPB, rows, :]
            else:
                ref = src.at[t // HPB, t % HPB, :, rows, :]
            return pltpu.make_async_copy(ref, buf.at[slot, :, pl.ds(c * R, R), :], sems.at[s0 + slot])

        def issue_kv(i, after_v=None):
            for c in range(NPC):
                kv_copy(k_hbm, kbuf, S_K, i, c).start(priority=0)
                if c + LV < NPC:
                    kv_copy(v_hbm, vbuf, S_V, i, c + LV).start(priority=1)
                elif after_v is None:
                    kv_copy(v_hbm, vbuf, S_V, i + 1, c + LV - NPC).start(priority=1)
                else:
                    after_v[c + LV - NPC].start(priority=1)

        def qpos(hq):
            if ST == 2:
                return (hq // 2 % 2) * QR + (hq // 4) * 2 + hq % 2
            return hq

        def wait_all(buf, s):
            pltpu.make_async_copy(buf, buf, sems.at[s]).wait()

        def block(fn):
            pl.when(flag[0] == 1)(fn)

        s0 = wcopies(wm_hbm, wm_buf, S_M, _pieces(0, NB_M, D // NB_M, 0, 6 * D, CW_M))
        s1 = wcopies(wq_hbm, wq_buf, S_Q, [p for b0, nb, cw in QS for p in _pieces(b0, nb, RB, 0, HQ * DH, cw)])
        s1 += [kv_copy(v_hbm, vbuf, S_V, 0, c) for c in range(LV)]
        lead = len(s1) - len(s0)
        small = [pltpu.make_async_copy(c_hbm, c_buf, sems.at[S_C]),
                 pltpu.make_async_copy(x_hbm, x_buf, sems.at[S_X]),
                 pltpu.make_async_copy(wr_hbm, wr_buf, sems.at[S_R])]
        for d in s1[:lead] + small:
            d.start(priority=1)
        for d0, d1 in zip(s0, s1[lead:]):
            d0.start(priority=0)
            d1.start(priority=1)

        def pre(i, carry):
            issue_kv(i)
            return carry

        jax.lax.fori_loop(0, 2, pre, 0)

        for d in small:
            d.wait()
        wait_all(wm_buf, S_M)
        c = c_buf[...].astype(f32)
        sc = (c * jax.nn.sigmoid(c)).astype(bf16)
        mod = jnp.dot(sc, wm_buf[...].reshape(D, 6 * D), preferred_element_type=f32)
        sa, ca, ga, sb, cb, gb = [mod[:, i * D:(i + 1) * D] for i in range(6)]
        x0 = x_buf[...].astype(f32)
        h1 = (_layernorm(x0) * (1.0 + ca) + sa).astype(bf16)

        block(lambda: issue_kv(2))
        wait_all(wq_buf, S_Q)
        for half in range(2):
            q = jnp.dot(h1, wq_buf[:, :, half * HW:(half + 1) * HW].reshape(D, HW), preferred_element_type=f32)
            for j in range(HQ // 2):
                q_all[:, qpos(half * (HQ // 2) + j), :] = q[:, j * DH:(j + 1) * DH]
            if 3 + half < DEPTH - 1:
                block(lambda: issue_kv(3 + half))
        assert DEPTH <= 6

        n_wo_loop = D // 8 - (LAG - LV) // 2
        gu_pieces = [p for b0, nb, cw in GU for p in _pieces(b0, nb, RB, 0, F, cw)]
        e0 = [wo_copy(8 * t, half) for t in range(n_wo_loop, D // 8) for half in range(2)]
        e0 += wcopies(wg_hbm, wg_buf, S_G, gu_pieces)
        e1 = wcopies(wu_hbm, wu_buf, S_U, gu_pieces)
        n_g = len(e0)
        for j, (bl, bh, cl, ch) in enumerate(STAGES):
            nb = (bh - bl) // 2
            if nb:
                cw = CW_A if nb > 1 else F // 2
                e0 += wcopies(wd_hbm, wd_buf, S_D + j, _pieces(bl, nb, RB, cl, ch, cw))
                e1 += wcopies(wd_hbm, wd_buf, S_D + j, _pieces(bl + nb, nb, RB, cl, ch, cw))
            else:
                ps = wcopies(wd_hbm, wd_buf, S_D + j, _pieces(bl, 1, RB, cl, ch, ch - cl))
                e0 += ps[:len(ps) // 2]
                e1 += ps[len(ps) // 2:]
        assert len(e0) + LV - len(e1) == pad_buf.shape[0]
        e1 += [pltpu.make_async_copy(wo_hbm.at[pl.ds(0, 8), pl.ds(128 * j, 128)], pad_buf.at[j], sems.at[S_PAD])
               for j in range(pad_buf.shape[0])]
        eseq = [x for d0, d1 in zip(e0, e1[LV:]) for x in ((d0, 0), (d1, 1))]

        def issue_range(lo, hi):
            for d, prio in eseq[lo:hi]:
                d.start(priority=prio)

        row_s = jax.lax.broadcasted_iota(jnp.int32, (QR, CH), 0) // 2
        row_o = jax.lax.broadcasted_iota(jnp.int32, (QR, DH), 0) // 2
        per_step = 2 * (CH // R)

        def superstep(t, carry):
            b = t // HPB
            q0 = pl.multiple_of((t % HPB) * QR, QR)
            qh = q_all[b, pl.ds(q0, QR), :].astype(bf16)

            def step(c, state):
                m, l, acc = state
                i = t * NC + c
                slot = i % DEPTH
                nxt = i + DEPTH - 1

                @pl.when(nxt < NSTEP - 1)
                def _():
                    issue_kv(nxt)

                @pl.when(nxt == NSTEP - 1)
                def _():
                    issue_kv(NSTEP - 1, e1[:LV])

                @pl.when(i < n_wo_loop)
                def _():
                    for half in range(2):
                        wo_copy(pl.multiple_of(i * 8, 8), half).start(priority=half)

                for e in range(DEPTH - 1):
                    @pl.when(nxt == NSTEP + e)
                    def _():
                        issue_range(e * per_step, (e + 1) * per_step)

                wait_all(kbuf.at[slot], S_K + slot)
                s = jax.lax.dot_general(qh, kbuf[slot, 0], NT, preferred_element_type=f32)
                for j in range(1, HG):
                    sj = jax.lax.dot_general(qh, kbuf[slot, j], NT, preferred_element_type=f32)
                    s = jnp.where(row_s == j, sj, s)
                m_new = jnp.maximum(m, jnp.max(s, axis=-1, keepdims=True))
                alpha = jnp.exp((m - m_new) * scale)
                p = jnp.exp((s - m_new) * scale)
                l = l * alpha + jnp.sum(p, axis=-1, keepdims=True)
                pb = p.astype(bf16)
                vslot = i % DV
                wait_all(vbuf.at[vslot], S_V + vslot)
                o = jnp.dot(pb, vbuf[vslot, 0], preferred_element_type=f32)
                for j in range(1, HG):
                    oj = jnp.dot(pb, vbuf[vslot, j], preferred_element_type=f32)
                    o = jnp.where(row_o == j, oj, o)
                return m_new, l, acc * alpha + o

            init = (jnp.full((QR, 1), -jnp.inf, f32), jnp.zeros((QR, 1), f32), jnp.zeros((QR, DH), f32))
            _, l, acc = jax.lax.fori_loop(0, NC, step, init)
            o_all[b, pl.ds(q0, QR), :] = acc / l
            return carry

        jax.lax.fori_loop(0, NS, superstep, 0)

        p0 = (DEPTH - 1) * per_step
        cuts = [p0, p0 + P_WO, p0 + P_WO + P_O2, 2 * n_g + P_G, 2 * n_g + P_G + P_U, len(eseq)]

        def issue_part(n):
            block(lambda: issue_range(cuts[n], cuts[n + 1]))

        issue_part(0)
        wait_all(wo_buf, S_O)
        attn = None
        for half in range(2):
            o_cat = jnp.concatenate([o_all[:, qpos(half * (HQ // 2) + j), :] for j in range(HQ // 2)], axis=1)
            part = jax.lax.dot_general(o_cat.astype(bf16), wo_buf[:, half * HW:(half + 1) * HW], NT,
                                       preferred_element_type=f32)
            if half == 0:
                attn = part
                issue_part(1)
            else:
                attn = attn + part
        x1 = x0 + ga * attn
        h2 = _layernorm(x1) * (1.0 + cb) + sb
        h2b = h2.astype(bf16)
        r = jnp.sum(h2 * wr_buf[...].astype(f32).reshape(1, D), axis=-1, keepdims=True)
        fin[0] = x1 + gb * h2
        fin[1] = gb * jax.nn.sigmoid(r)

        issue_part(2)
        wait_all(wg_buf, S_G)
        g = jnp.dot(h2b, wg_buf[...].reshape(D, F), preferred_element_type=f32)
        g = g * jax.nn.sigmoid(g)
        issue_part(3)
        wait_all(wu_buf, S_U)
        u = jnp.dot(h2b, wu_buf[...].reshape(D, F), preferred_element_type=f32)
        act = (g * u).astype(bf16)
        issue_part(4)

        for j, (bl, bh, cl, ch) in enumerate(STAGES):
            view = (pl.ds(bl, bh - bl), slice(None), pl.ds(cl, ch - cl))
            lo, hi = bl * RB, bh * RB
            wait_all(wd_buf.at[view], S_D + j)
            y = jax.lax.dot_general(act[:, cl:ch], wd_buf[view].reshape(hi - lo, ch - cl), NT,
                                    preferred_element_type=f32)
            res = fin[0, :, lo:hi] + fin[1, :, lo:hi] * y
            if ch == F:
                out_ref[:, lo:hi] = res.astype(out_ref.dtype)
            else:
                fin[0, :, lo:hi] = res
        wait_all(pad_buf, S_PAD)

    @jax.jit
    def fn(A_x, A_k_cache, A_v_cache, A_wq, A_wo, B_x, B_w_r, B_w_gate, B_w_up, B_w_down, c, w_mod):
        SK = A_k_cache.shape[2]
        kv_shape = (B, HG, HKV // HG, SK, DH) if ST == 2 else (B, HKV // HG, HG, SK, DH)
        out = pl.pallas_call(
            kernel,
            out_shape=jax.ShapeDtypeStruct((B, D), bf16),
            in_specs=[pl.BlockSpec(memory_space=pl.ANY)] * 11,
            out_specs=pl.BlockSpec(memory_space=pltpu.VMEM),
            scratch_shapes=[
                pltpu.VMEM((B, D), bf16), pltpu.VMEM((B, D), bf16), pltpu.VMEM((D,), bf16),
                pltpu.VMEM((NB_M, D // NB_M, 6 * D), bf16), pltpu.VMEM((NB, RB, HQ * DH), bf16),
                pltpu.VMEM((D, HQ * DH), bf16),
                pltpu.VMEM((NB, RB, F), bf16), pltpu.VMEM((NB, RB, F), bf16), pltpu.VMEM((NB, RB, F), bf16),
                pltpu.VMEM(((LAG - LV) // 2 * 2 + LV, 8, 128), bf16),
                pltpu.VMEM((DEPTH, HG, CH, DH), bf16), pltpu.VMEM((DV, HG, CH, DH), bf16),
                pltpu.VMEM((B, HQ, DH), f32), pltpu.VMEM((B, HQ, DH), f32), pltpu.VMEM((2, B, D), f32),
                pltpu.SMEM((1,), jnp.int32), pltpu.SemaphoreType.DMA((S_V + DV,)),
            ],
            compiler_params=pltpu.CompilerParams(vmem_limit_bytes=64 * 1024 * 1024,
                                                 disable_bounds_checks=not check,
                                                 disable_semaphore_checks=not check),
        )(A_x.reshape(B, D), A_k_cache.reshape(kv_shape), A_v_cache.reshape(kv_shape), A_wq.reshape(NB, RB, HQ * DH), A_wo.T, B_w_r,
          B_w_gate.reshape(NB, RB, F), B_w_up.reshape(NB, RB, F), B_w_down.T.reshape(NB, RB, F),
          c, w_mod.reshape(NB_M, D // NB_M, 6 * D))
        return out.reshape(B, 1, D)

    return fn


pallas_adaLN_cond__sliding_block_cached__moe_arch_mod__decode_kernel = build()
```

```python
import jax
import jax.numpy as jnp
import jax.experimental.pallas as pl
import jax.experimental.pallas.tpu as pltpu

B, D = 8, 576
HQ, HKV, DH = 32, 16, 128
F = 4608
EPS = 1e-05
NT = (((1,), (1,)), ((), ()))
f32 = jnp.float32
bf16 = jnp.bfloat16

HG, CH, R = 8, 256, 16
NPC = CH // R
QR = 2 * HG
HPB = HKV // HG
DK = 4
DV = DK + 1
LV = 2
LAG = 26
NB_M, NB = 4, 9
RB = D // NB
HW = HQ * DH // 2
STAGES = ((0, 6, 0, F, 768), (6, 8, 0, F, F // 2), (8, 9, 0, 2816, 2816), (8, 9, 2816, F, F - 2816))
S_C, S_X, S_R, S_PAD, S_M, S_Q, S_O, S_G, S_U, S_D = range(10)
S_K = S_D + len(STAGES)
S_V = S_K + DK


def _layernorm(x):
    m = jnp.mean(x, axis=-1, keepdims=True)
    xc = x - m
    v = jnp.mean(xc * xc, axis=-1, keepdims=True)
    return xc / jnp.sqrt(v + EPS)


def _qpos(hq):
    return (hq // 2 % 2) * QR + (hq // 4) * 2 + hq % 2


def _kernel(x_hbm, k_hbm, v_hbm, wq_hbm, wo_hbm, wr_hbm, wg_hbm, wu_hbm, wd_hbm, c_hbm, wm_hbm,
            out_ref,
            x_buf, c_buf, wr_buf, wm_buf, wq_buf, wo_buf, wg_buf, wu_buf, wd_buf, pad_buf,
            kbuf, vbuf, q_all, o_all, fin, flag, sems):
    SK = k_hbm.shape[3]
    W = min(4096, max(256, SK // 4))
    NC = W // CH
    NS = B * HPB
    NSTEP = NS * NC
    scale = DH ** -0.5
    flag[0] = 1

    def wcopies(src, dst, s, *specs):
        out = []
        for b0, nb, c_lo, c_hi, cw in specs:
            for r in range(0, src.shape[1], 8):
                for c0 in range(c_lo, c_hi, cw):
                    idx = (pl.ds(b0, nb), pl.ds(r, 8), pl.ds(c0, min(cw, c_hi - c0)))
                    out.append(pltpu.make_async_copy(src.at[idx], dst.at[idx], sems.at[s]))
        return out

    def kv_copy(src, buf, s0, i, c):
        t = i // NC
        rows = pl.ds(pl.multiple_of(SK - W + (i % NC) * CH + c * R, R), R)
        slot = i % buf.shape[0]
        return pltpu.make_async_copy(src.at[t // HPB, :, t % HPB, rows, :],
                                     buf.at[slot, :, pl.ds(c * R, R), :], sems.at[s0 + slot])

    def k_copies(i):
        return [kv_copy(k_hbm, kbuf, S_K, i, c) for c in range(NPC)]

    def v_copies(i, n=NPC):
        return [kv_copy(v_hbm, vbuf, S_V, i + (c + LV) // NPC, (c + LV) % NPC) for c in range(n)]

    def interleave(l0, l1):
        assert len(l0) == len(l1)
        return [x for d0, d1 in zip(l0, l1) for x in ((d0, 0), (d1, 1))]

    def issue(seq):
        for d, prio in seq:
            d.start(priority=prio)

    def issue_block(seq):
        @pl.when(flag[0] == 1)
        def _():
            issue(seq)

    def wait_all(buf, s):
        pltpu.make_async_copy(buf, buf, sems.at[s]).wait()

    qo_specs = ((0, 1, 0, 2 * HW, HW), (1, 8, 0, 2 * HW, 256))
    wo_all = wcopies(wo_hbm, wo_buf, S_O, *qo_specs)
    n_late = LAG - LV
    s0 = wcopies(wm_hbm, wm_buf, S_M, (0, 2, 0, 6 * D, 1024))
    s1 = wcopies(wm_hbm, wm_buf, S_M, (2, 2, 0, 6 * D, 1024))
    n_m = len(s0)
    s0 += wo_all[:-n_late]
    s1 += wcopies(wq_hbm, wq_buf, S_Q, *qo_specs)
    s1 += [kv_copy(v_hbm, vbuf, S_V, 0, c) for c in range(LV)]
    for i in range(DK - 1):
        s0 += k_copies(i)
        s1 += v_copies(i)
    small = [pltpu.make_async_copy(c_hbm, c_buf, sems.at[S_C]),
             pltpu.make_async_copy(x_hbm, x_buf, sems.at[S_X]),
             pltpu.make_async_copy(wr_hbm, wr_buf, sems.at[S_R])]
    sseq = [(d, 1) for d in s1[:LAG]] + [(d, 0) for d in small] + interleave(s0, s1[LAG:])
    cut = LAG + len(small) + 2 * n_m + 70

    issue(sseq[:cut])
    for d in small:
        d.wait()
    wait_all(wm_buf, S_M)
    c = c_buf[...].astype(f32)
    sc = (c * jax.nn.sigmoid(c)).astype(bf16)
    mod = jnp.dot(sc, wm_buf[...].reshape(D, 6 * D), preferred_element_type=f32)
    sa, ca, ga, sb, cb, gb = [mod[:, i * D:(i + 1) * D] for i in range(6)]
    x0 = x_buf[...].astype(f32)
    h1 = (_layernorm(x0) * (1.0 + ca) + sa).astype(bf16)

    issue_block(sseq[cut:])
    wait_all(wq_buf, S_Q)
    q = jnp.dot(h1, wq_buf[...].reshape(D, HQ * DH), preferred_element_type=f32)
    for hq in range(HQ):
        q_all[:, _qpos(hq), :] = q[:, hq * DH:(hq + 1) * DH]

    gu_specs = ((0, 5, 0, F, 384), (5, 4, 0, F, 512))
    e0 = wo_all[-n_late:] + wcopies(wg_hbm, wg_buf, S_G, *gu_specs)
    e1 = wcopies(wu_hbm, wu_buf, S_U, *gu_specs)
    n_g = len(e0)
    for j, (bl, bh, cl, ch, cw) in enumerate(STAGES):
        nb = (bh - bl) // 2
        if nb:
            e0 += wcopies(wd_hbm, wd_buf, S_D + j, (bl, nb, cl, ch, cw))
            e1 += wcopies(wd_hbm, wd_buf, S_D + j, (bl + nb, nb, cl, ch, cw))
        else:
            ps = wcopies(wd_hbm, wd_buf, S_D + j, (bl, 1, cl, ch, cw))
            e0 += ps[:len(ps) // 2]
            e1 += ps[len(ps) // 2:]
    e1 += [pltpu.make_async_copy(wo_hbm.at[0, pl.ds(0, 8), pl.ds(128 * j, 128)], pad_buf.at[j], sems.at[S_PAD])
           for j in range(LAG)]
    eseq = interleave(e0, e1[LV:])

    row_s = jax.lax.broadcasted_iota(jnp.int32, (QR, CH), 0) // 2
    row_o = jax.lax.broadcasted_iota(jnp.int32, (QR, DH), 0) // 2

    def group(t, carry):
        b = t // HPB
        q0 = pl.multiple_of((t % HPB) * QR, QR)
        qh = q_all[b, pl.ds(q0, QR), :].astype(bf16)

        def step(cidx, state):
            m, l, acc = state
            i = t * NC + cidx
            nxt = i + DK - 1

            @pl.when(nxt < NSTEP - 1)
            def _():
                issue(interleave(k_copies(nxt), v_copies(nxt)))

            @pl.when(nxt == NSTEP - 1)
            def _():
                issue(interleave(k_copies(NSTEP - 1), v_copies(NSTEP - 1, NPC - LV) + e1[:LV]))

            for e in range(DK - 1):
                @pl.when(nxt == NSTEP + e)
                def _():
                    issue(eseq[e * 2 * NPC:(e + 1) * 2 * NPC])

            ks = i % DK
            wait_all(kbuf.at[ks], S_K + ks)
            s = jax.lax.dot_general(qh, kbuf[ks, 0], NT, preferred_element_type=f32)
            for j in range(1, HG):
                sj = jax.lax.dot_general(qh, kbuf[ks, j], NT, preferred_element_type=f32)
                s = jnp.where(row_s == j, sj, s)
            m_new = jnp.maximum(m, jnp.max(s, axis=-1, keepdims=True))
            alpha = jnp.exp((m - m_new) * scale)
            p = jnp.exp((s - m_new) * scale)
            l = l * alpha + jnp.sum(p, axis=-1, keepdims=True)
            pb = p.astype(bf16)
            vs = i % DV
            wait_all(vbuf.at[vs], S_V + vs)
            o = jnp.dot(pb, vbuf[vs, 0], preferred_element_type=f32)
            for j in range(1, HG):
                oj = jnp.dot(pb, vbuf[vs, j], preferred_element_type=f32)
                o = jnp.where(row_o == j, oj, o)
            return m_new, l, acc * alpha + o

        init = (jnp.full((QR, 1), -jnp.inf, f32), jnp.zeros((QR, 1), f32), jnp.zeros((QR, DH), f32))
        _, l, acc = jax.lax.fori_loop(0, NC, step, init)
        o_all[b, pl.ds(q0, QR), :] = acc / l
        return carry

    jax.lax.fori_loop(0, NS, group, 0)

    p0 = (DK - 1) * 2 * NPC
    cuts = [p0, p0 + 40, p0 + 70, 2 * n_g + 70, 2 * n_g + 80, len(eseq)]

    issue_block(eseq[cuts[0]:cuts[1]])
    wait_all(wo_buf, S_O)
    parts = []
    for half in range(2):
        o_cat = jnp.concatenate([o_all[:, _qpos(half * (HQ // 2) + j), :] for j in range(HQ // 2)], axis=1)
        parts.append(jax.lax.dot_general(o_cat.astype(bf16),
                                         wo_buf[:, :, half * HW:(half + 1) * HW].reshape(D, HW), NT,
                                         preferred_element_type=f32))
        if half == 0:
            issue_block(eseq[cuts[1]:cuts[2]])
    x1 = x0 + ga * (parts[0] + parts[1])
    h2 = _layernorm(x1) * (1.0 + cb) + sb
    h2b = h2.astype(bf16)
    r = jnp.sum(h2 * wr_buf[...].astype(f32).reshape(1, D), axis=-1, keepdims=True)
    fin[0] = x1 + gb * h2
    fin[1] = gb * jax.nn.sigmoid(r)

    issue_block(eseq[cuts[2]:cuts[3]])
    wait_all(wg_buf, S_G)
    g = jnp.dot(h2b, wg_buf[...].reshape(D, F), preferred_element_type=f32)
    g = g * jax.nn.sigmoid(g)
    issue_block(eseq[cuts[3]:cuts[4]])
    wait_all(wu_buf, S_U)
    u = jnp.dot(h2b, wu_buf[...].reshape(D, F), preferred_element_type=f32)
    act = (g * u).astype(bf16)
    issue_block(eseq[cuts[4]:cuts[5]])

    for j, (bl, bh, cl, ch, _) in enumerate(STAGES):
        view = (pl.ds(bl, bh - bl), slice(None), pl.ds(cl, ch - cl))
        lo, hi = bl * RB, bh * RB
        wait_all(wd_buf.at[view], S_D + j)
        y = jax.lax.dot_general(act[:, cl:ch], wd_buf[view].reshape(hi - lo, ch - cl), NT,
                                preferred_element_type=f32)
        res = fin[0, :, lo:hi] + fin[1, :, lo:hi] * y
        if ch == F:
            out_ref[:, lo:hi] = res.astype(out_ref.dtype)
        else:
            fin[0, :, lo:hi] = res
    wait_all(pad_buf, S_PAD)


@jax.jit
def pallas_adaLN_cond__sliding_block_cached__moe_arch_mod__decode_kernel(
    A_x: jax.Array,
    A_k_cache: jax.Array,
    A_v_cache: jax.Array,
    A_wq: jax.Array,
    A_wo: jax.Array,
    B_x: jax.Array,
    B_w_r: jax.Array,
    B_w_gate: jax.Array,
    B_w_up: jax.Array,
    B_w_down: jax.Array,
    c: jax.Array,
    w_mod: jax.Array,
):
    kv_shape = (B, HG, HPB, A_k_cache.shape[2], DH)
    out = pl.pallas_call(
        _kernel,
        out_shape=jax.ShapeDtypeStruct((B, D), bf16),
        in_specs=[pl.BlockSpec(memory_space=pl.ANY)] * 11,
        out_specs=pl.BlockSpec(memory_space=pltpu.VMEM),
        scratch_shapes=[
            pltpu.VMEM((B, D), bf16), pltpu.VMEM((B, D), bf16), pltpu.VMEM((D,), bf16),
            pltpu.VMEM((NB_M, D // NB_M, 6 * D), bf16),
            pltpu.VMEM((NB, RB, HQ * DH), bf16), pltpu.VMEM((NB, RB, HQ * DH), bf16),
            pltpu.VMEM((NB, RB, F), bf16), pltpu.VMEM((NB, RB, F), bf16), pltpu.VMEM((NB, RB, F), bf16),
            pltpu.VMEM((LAG, 8, 128), bf16),
            pltpu.VMEM((DK, HG, CH, DH), bf16), pltpu.VMEM((DV, HG, CH, DH), bf16),
            pltpu.VMEM((B, HQ, DH), f32), pltpu.VMEM((B, HQ, DH), f32), pltpu.VMEM((2, B, D), f32),
            pltpu.SMEM((1,), jnp.int32), pltpu.SemaphoreType.DMA((S_V + DV,)),
        ],
        compiler_params=pltpu.CompilerParams(vmem_limit_bytes=64 * 1024 * 1024,
                                             disable_bounds_checks=True,
                                             disable_semaphore_checks=True),
    )(A_x.reshape(B, D), A_k_cache.reshape(kv_shape), A_v_cache.reshape(kv_shape),
      A_wq.reshape(NB, RB, HQ * DH), A_wo.T.reshape(NB, RB, HQ * DH), B_w_r,
      B_w_gate.reshape(NB, RB, F), B_w_up.reshape(NB, RB, F), B_w_down.T.reshape(NB, RB, F),
      c, w_mod.reshape(NB_M, D // NB_M, 6 * D))
    return out.reshape(B, 1, D)
```

```python
import jax
import jax.numpy as jnp
import jax.experimental.pallas as pl
import jax.experimental.pallas.tpu as pltpu

B, D = 8, 576
HQ, HKV, DH = 32, 16, 128
F = 4608
EPS = 1e-05
NT = (((1,), (1,)), ((), ()))
f32 = jnp.float32
bf16 = jnp.bfloat16

HG, CH, R = 8, 256, 16
NPC = CH // R
QR = 2 * HG
HPB = HKV // HG
DK = 4
DV = DK + 1
LV = 2
LAG = 26
NB_M, NB = 4, 9
RB = D // NB
HW = HQ * DH // 2
CS = 3072
STAGES = ((0, 6, 0, F, 768), (6, 8, 0, F, F // 2), (8, 9, 0, CS, CS), (8, 9, CS, F, F - CS))
S_C, S_X, S_R, S_PAD, S_M, S_Q, S_O, S_G, S_U, S_OUT0, S_OUT1, S_D = range(12)
S_K = S_D + len(STAGES)
S_V = S_K + DK


def _layernorm(x):
    m = jnp.mean(x, axis=-1, keepdims=True)
    xc = x - m
    v = jnp.mean(xc * xc, axis=-1, keepdims=True)
    return xc / jnp.sqrt(v + EPS)


def _qpos(hq):
    return (hq // 2 % 2) * QR + (hq // 4) * 2 + hq % 2


def _kernel(x_hbm, k_hbm, v_hbm, wq_hbm, wo_hbm, wr_hbm, wg_hbm, wu_hbm, wd_hbm, c_hbm, wm_hbm,
            out_hbm,
            x_buf, c_buf, wr_buf, wm_buf, wq_buf, wo_buf, wg_buf, wu_buf, wd_buf, pad_buf,
            kbuf, vbuf, q_all, o_all, fin, out_buf, flag, sems):
    SK = k_hbm.shape[3]
    W = min(4096, max(256, SK // 4))
    NC = W // CH
    NS = B * HPB
    NSTEP = NS * NC
    scale = DH ** -0.5
    flag[0] = 1

    def wcopies(src, dst, s, *specs):
        out = []
        for b0, nb, c_lo, c_hi, cw in specs:
            for r in range(0, src.shape[1], 8):
                for c0 in range(c_lo, c_hi, cw):
                    idx = (pl.ds(b0, nb), pl.ds(r, 8), pl.ds(c0, min(cw, c_hi - c0)))
                    out.append(pltpu.make_async_copy(src.at[idx], dst.at[idx], sems.at[s]))
        return out

    def kv_copy(src, buf, s0, i, c):
        t = i // NC
        rows = pl.ds(pl.multiple_of(SK - W + (i % NC) * CH + c * R, R), R)
        slot = i % buf.shape[0]
        return pltpu.make_async_copy(src.at[t // HPB, :, t % HPB, rows, :],
                                     buf.at[slot, :, pl.ds(c * R, R), :], sems.at[s0 + slot])

    def k_copies(i):
        return [kv_copy(k_hbm, kbuf, S_K, i, c) for c in range(NPC)]

    def v_copies(i, n=NPC):
        return [kv_copy(v_hbm, vbuf, S_V, i + (c + LV) // NPC, (c + LV) % NPC) for c in range(n)]

    def interleave(l0, l1):
        assert len(l0) == len(l1)
        return [x for d0, d1 in zip(l0, l1) for x in ((d0, 0), (d1, 1))]

    def issue(seq):
        for d, prio in seq:
            d.start(priority=prio)

    def issue_block(seq):
        @pl.when(flag[0] == 1)
        def _():
            issue(seq)

    def wait_all(buf, s):
        pltpu.make_async_copy(buf, buf, sems.at[s]).wait()

    qo_specs = ((0, 1, 0, 2 * HW, HW), (1, 8, 0, 2 * HW, 256))
    wo_all = wcopies(wo_hbm, wo_buf, S_O, *qo_specs)
    n_late = LAG - LV
    s0 = wcopies(wm_hbm, wm_buf, S_M, (0, 2, 0, 6 * D, 1152))
    s1 = wcopies(wm_hbm, wm_buf, S_M, (2, 2, 0, 6 * D, 1152))
    n_m = len(s0)
    s0 += wo_all[:-n_late]
    s1 += wcopies(wq_hbm, wq_buf, S_Q, *qo_specs)
    s1 += [kv_copy(v_hbm, vbuf, S_V, 0, c) for c in range(LV)]
    for i in range(DK - 1):
        s0 += k_copies(i)
        s1 += v_copies(i)
    small = [pltpu.make_async_copy(c_hbm, c_buf, sems.at[S_C]),
             pltpu.make_async_copy(x_hbm, x_buf, sems.at[S_X]),
             pltpu.make_async_copy(wr_hbm, wr_buf, sems.at[S_R])]
    sseq = [(d, 1) for d in s1[:LAG]] + [(d, 0) for d in small] + interleave(s0, s1[LAG:])
    cut = LAG + len(small) + 2 * n_m + 70

    issue(sseq[:cut])
    for d in small:
        d.wait()
    wait_all(wm_buf, S_M)
    c = c_buf[...].astype(f32)
    sc = (c * jax.nn.sigmoid(c)).astype(bf16)
    mod = jnp.dot(sc, wm_buf[...].reshape(D, 6 * D), preferred_element_type=f32)
    sa, ca, ga, sb, cb, gb = [mod[:, i * D:(i + 1) * D] for i in range(6)]
    x0 = x_buf[...].astype(f32)
    h1 = (_layernorm(x0) * (1.0 + ca) + sa).astype(bf16)

    issue_block(sseq[cut:])
    wait_all(wq_buf, S_Q)
    q = jnp.dot(h1, wq_buf[...].reshape(D, HQ * DH), preferred_element_type=f32)
    for hq in range(HQ):
        q_all[:, _qpos(hq), :] = q[:, hq * DH:(hq + 1) * DH]

    gu_specs = ((5, 4, 0, F, 512), (0, 5, 0, F, 384))
    e0 = wo_all[-n_late:] + wcopies(wg_hbm, wg_buf, S_G, *gu_specs)
    e1 = wcopies(wu_hbm, wu_buf, S_U, *gu_specs)
    n_g = len(e0)
    for j, (bl, bh, cl, ch, cw) in enumerate(STAGES):
        nb = (bh - bl) // 2
        if nb:
            e0 += wcopies(wd_hbm, wd_buf, S_D + j, (bl, nb, cl, ch, cw))
            e1 += wcopies(wd_hbm, wd_buf, S_D + j, (bl + nb, nb, cl, ch, cw))
        else:
            ps = wcopies(wd_hbm, wd_buf, S_D + j, (bl, 1, cl, ch, cw))
            e0 += ps[:len(ps) // 2]
            e1 += ps[len(ps) // 2:]
    e1 += [pltpu.make_async_copy(wo_hbm.at[0, pl.ds(0, 8), pl.ds(128 * j, 128)], pad_buf.at[j], sems.at[S_PAD])
           for j in range(LAG)]
    eseq = interleave(e0, e1[LV:])

    row_s = jax.lax.broadcasted_iota(jnp.int32, (QR, CH), 0) // 2
    row_o = jax.lax.broadcasted_iota(jnp.int32, (QR, DH), 0) // 2

    def group(t, carry):
        b = t // HPB
        q0 = pl.multiple_of((t % HPB) * QR, QR)
        qh = q_all[b, pl.ds(q0, QR), :].astype(bf16)

        def step(cidx, state):
            m, l, acc = state
            i = t * NC + cidx
            nxt = i + DK - 1

            @pl.when(nxt < NSTEP - 1)
            def _():
                issue(interleave(k_copies(nxt), v_copies(nxt)))

            @pl.when(nxt == NSTEP - 1)
            def _():
                issue(interleave(k_copies(NSTEP - 1), v_copies(NSTEP - 1, NPC - LV) + e1[:LV]))

            for e in range(DK - 1):
                @pl.when(nxt == NSTEP + e)
                def _():
                    issue(eseq[e * 2 * NPC:(e + 1) * 2 * NPC])

            ks = i % DK
            wait_all(kbuf.at[ks], S_K + ks)
            s = jax.lax.dot_general(qh, kbuf[ks, 0], NT, preferred_element_type=f32)
            for j in range(1, HG):
                sj = jax.lax.dot_general(qh, kbuf[ks, j], NT, preferred_element_type=f32)
                s = jnp.where(row_s == j, sj, s)
            m_new = jnp.maximum(m, jnp.max(s, axis=-1, keepdims=True))
            alpha = jnp.exp((m - m_new) * scale)
            p = jnp.exp((s - m_new) * scale)
            l = l * alpha + jnp.sum(p, axis=-1, keepdims=True)
            pb = p.astype(bf16)
            vs = i % DV
            wait_all(vbuf.at[vs], S_V + vs)
            o = jnp.dot(pb, vbuf[vs, 0], preferred_element_type=f32)
            for j in range(1, HG):
                oj = jnp.dot(pb, vbuf[vs, j], preferred_element_type=f32)
                o = jnp.where(row_o == j, oj, o)
            return m_new, l, acc * alpha + o

        init = (jnp.full((QR, 1), -jnp.inf, f32), jnp.zeros((QR, 1), f32), jnp.zeros((QR, DH), f32))
        _, l, acc = jax.lax.fori_loop(0, NC, step, init)
        o_all[b, pl.ds(q0, QR), :] = acc / l
        return carry

    jax.lax.fori_loop(0, NS, group, 0)

    p0 = (DK - 1) * 2 * NPC
    cuts = [p0, p0 + 40, p0 + 70, 2 * n_g + 70, 2 * n_g + 80, len(eseq)]

    issue_block(eseq[cuts[0]:cuts[1]])
    wait_all(wo_buf, S_O)
    parts = []
    for half in range(2):
        o_cat = jnp.concatenate([o_all[:, _qpos(half * (HQ // 2) + j), :] for j in range(HQ // 2)], axis=1)
        parts.append(jax.lax.dot_general(o_cat.astype(bf16),
                                         wo_buf[:, :, half * HW:(half + 1) * HW].reshape(D, HW), NT,
                                         preferred_element_type=f32))
        if half == 0:
            issue_block(eseq[cuts[1]:cuts[2]])
    x1 = x0 + ga * (parts[0] + parts[1])
    h2 = _layernorm(x1) * (1.0 + cb) + sb
    h2b = h2.astype(bf16)
    r = jnp.sum(h2 * wr_buf[...].astype(f32).reshape(1, D), axis=-1, keepdims=True)
    fin[0] = x1 + gb * h2
    fin[1] = gb * jax.nn.sigmoid(r)

    issue_block(eseq[cuts[2]:cuts[3]])
    wait_all(wg_buf, S_G)
    g = jnp.dot(h2b, wg_buf[...].reshape(D, F), preferred_element_type=f32)
    g = g * jax.nn.sigmoid(g)
    issue_block(eseq[cuts[3]:cuts[4]])
    wait_all(wu_buf, S_U)
    u = jnp.dot(h2b, wu_buf[...].reshape(D, F), preferred_element_type=f32)
    act = (g * u).astype(bf16)
    issue_block(eseq[cuts[4]:cuts[5]])

    n_early = STAGES[-1][0] * RB
    out_cps = [pltpu.make_async_copy(out_buf.at[:, pl.ds(c0, cn)], out_hbm.at[:, pl.ds(c0, cn)], sems.at[s])
               for c0, cn, s in ((0, n_early, S_OUT0), (n_early, D - n_early, S_OUT1))]
    for j, (bl, bh, cl, ch, _) in enumerate(STAGES):
        view = (pl.ds(bl, bh - bl), slice(None), pl.ds(cl, ch - cl))
        lo, hi = bl * RB, bh * RB
        wait_all(wd_buf.at[view], S_D + j)
        y = jax.lax.dot_general(act[:, cl:ch], wd_buf[view].reshape(hi - lo, ch - cl), NT,
                                preferred_element_type=f32)
        res = fin[0, :, lo:hi] + fin[1, :, lo:hi] * y
        if ch == F:
            out_buf[:, lo:hi] = res.astype(bf16)
            if hi == n_early:
                out_cps[0].start()
        else:
            fin[0, :, lo:hi] = res
    out_cps[1].start()
    wait_all(pad_buf, S_PAD)
    out_cps[0].wait()
    out_cps[1].wait()


@jax.jit
def pallas_adaLN_cond__sliding_block_cached__moe_arch_mod__decode_kernel(
    A_x: jax.Array,
    A_k_cache: jax.Array,
    A_v_cache: jax.Array,
    A_wq: jax.Array,
    A_wo: jax.Array,
    B_x: jax.Array,
    B_w_r: jax.Array,
    B_w_gate: jax.Array,
    B_w_up: jax.Array,
    B_w_down: jax.Array,
    c: jax.Array,
    w_mod: jax.Array,
):
    kv_shape = (B, HG, HPB, A_k_cache.shape[2], DH)
    out = pl.pallas_call(
        _kernel,
        out_shape=jax.ShapeDtypeStruct((B, D), bf16),
        in_specs=[pl.BlockSpec(memory_space=pl.ANY)] * 11,
        out_specs=pl.BlockSpec(memory_space=pl.ANY),
        scratch_shapes=[
            pltpu.VMEM((B, D), bf16), pltpu.VMEM((B, D), bf16), pltpu.VMEM((D,), bf16),
            pltpu.VMEM((NB_M, D // NB_M, 6 * D), bf16),
            pltpu.VMEM((NB, RB, HQ * DH), bf16), pltpu.VMEM((NB, RB, HQ * DH), bf16),
            pltpu.VMEM((NB, RB, F), bf16), pltpu.VMEM((NB, RB, F), bf16), pltpu.VMEM((NB, RB, F), bf16),
            pltpu.VMEM((LAG, 8, 128), bf16),
            pltpu.VMEM((DK, HG, CH, DH), bf16), pltpu.VMEM((DV, HG, CH, DH), bf16),
            pltpu.VMEM((B, HQ, DH), f32), pltpu.VMEM((B, HQ, DH), f32), pltpu.VMEM((2, B, D), f32),
            pltpu.VMEM((B, D), bf16),
            pltpu.SMEM((1,), jnp.int32), pltpu.SemaphoreType.DMA((S_V + DV,)),
        ],
        compiler_params=pltpu.CompilerParams(vmem_limit_bytes=64 * 1024 * 1024,
                                             disable_bounds_checks=True,
                                             disable_semaphore_checks=True),
    )(A_x.reshape(B, D), A_k_cache.reshape(kv_shape), A_v_cache.reshape(kv_shape),
      A_wq.reshape(NB, RB, HQ * DH), A_wo.T.reshape(NB, RB, HQ * DH), B_w_r,
      B_w_gate.reshape(NB, RB, F), B_w_up.reshape(NB, RB, F), B_w_down.T.reshape(NB, RB, F),
      c, w_mod.reshape(NB_M, D // NB_M, 6 * D))
    return out.reshape(B, 1, D)
```

```python
import jax
import jax.numpy as jnp
import jax.experimental.pallas as pl
import jax.experimental.pallas.tpu as pltpu

B, D = 8, 576
HQ, HKV, DH = 32, 16, 128
F = 4608
EPS = 1e-05
NT = (((1,), (1,)), ((), ()))
f32 = jnp.float32
bf16 = jnp.bfloat16

HG, CH, R = 8, 256, 16
NPC = CH // R
QR = 2 * HG
HPB = HKV // HG
DK = 4
DV = DK + 1
LV = 2
LAG = 26
NB_M, NB = 4, 9
RB = D // NB
HW = HQ * DH // 2
CS = 3072
STAGES = ((0, 6, 0, F, 768), (6, 8, 0, F, F // 2), (8, 9, 0, CS, CS), (8, 9, CS, F, F - CS))
S_C, S_X, S_R, S_PAD, S_M, S_Q, S_O, S_G, S_U, S_OUT0, S_OUT1, S_D = range(12)
S_K = S_D + len(STAGES)
S_V = S_K + DK


def _layernorm(x):
    m = jnp.mean(x, axis=-1, keepdims=True)
    xc = x - m
    v = jnp.mean(xc * xc, axis=-1, keepdims=True)
    return xc / jnp.sqrt(v + EPS)


def _qpos(hq):
    return (hq // 2 % 2) * QR + (hq // 4) * 2 + hq % 2


def _kernel(x_hbm, k_hbm, v_hbm, wq_hbm, wo_hbm, wr_hbm, wg_hbm, wu_hbm, wd_hbm, c_hbm, wm_hbm,
            out_hbm,
            x_buf, c_buf, wr_buf, wm_buf, wq_buf, wo_buf, wg_buf, wu_buf, wd_buf, pad_buf,
            kbuf, vbuf, q_all, o_all, fin, out_buf, sems):
    SK = k_hbm.shape[3]
    W = min(4096, max(256, SK // 4))
    NC = W // CH
    NS = B * HPB
    NSTEP = NS * NC
    scale = DH ** -0.5

    def wcopies(src, dst, s, *specs):
        out = []
        for b0, nb, c_lo, c_hi, cw in specs:
            for r in range(0, src.shape[1], 8):
                for c0 in range(c_lo, c_hi, cw):
                    idx = (pl.ds(b0, nb), pl.ds(r, 8), pl.ds(c0, min(cw, c_hi - c0)))
                    out.append(pltpu.make_async_copy(src.at[idx], dst.at[idx], sems.at[s]))
        return out

    def kv_copy(src, buf, s0, i, c):
        t = i // NC
        rows = pl.ds(pl.multiple_of(SK - W + (i % NC) * CH + c * R, R), R)
        slot = i % buf.shape[0]
        return pltpu.make_async_copy(src.at[t // HPB, :, t % HPB, rows, :],
                                     buf.at[slot, :, pl.ds(c * R, R), :], sems.at[s0 + slot])

    def k_copies(i):
        return [kv_copy(k_hbm, kbuf, S_K, i, c) for c in range(NPC)]

    def v_copies(i, n=NPC):
        return [kv_copy(v_hbm, vbuf, S_V, i + (c + LV) // NPC, (c + LV) % NPC) for c in range(n)]

    def interleave(l0, l1):
        assert len(l0) == len(l1)
        return [x for d0, d1 in zip(l0, l1) for x in ((d0, 0), (d1, 1))]

    def issue(seq):
        for d, prio in seq:
            d.start(priority=prio)

    def issue_block(seq):
        half = (len(seq) + 1) // 2

        def body(it, carry):
            @pl.when(it == 0)
            def _():
                issue(seq[:half])

            @pl.when(it == 1)
            def _():
                issue(seq[half:])
            return carry

        jax.lax.fori_loop(0, 2, body, 0)

    def wait_all(buf, s):
        pltpu.make_async_copy(buf, buf, sems.at[s]).wait()

    qo_specs = ((0, 1, 0, 2 * HW, HW), (1, 8, 0, 2 * HW, 256))
    wo_all = wcopies(wo_hbm, wo_buf, S_O, *qo_specs)
    n_late = LAG - LV
    s0 = wcopies(wm_hbm, wm_buf, S_M, (0, 2, 0, 6 * D, 1152))
    s1 = wcopies(wm_hbm, wm_buf, S_M, (2, 2, 0, 6 * D, 1152))
    n_m = len(s0)
    s0 += wo_all[:-n_late]
    s1 += wcopies(wq_hbm, wq_buf, S_Q, *qo_specs)
    s1 += [kv_copy(v_hbm, vbuf, S_V, 0, c) for c in range(LV)]
    for i in range(DK - 1):
        s0 += k_copies(i)
        s1 += v_copies(i)
    small = [pltpu.make_async_copy(c_hbm, c_buf, sems.at[S_C]),
             pltpu.make_async_copy(x_hbm, x_buf, sems.at[S_X]),
             pltpu.make_async_copy(wr_hbm, wr_buf, sems.at[S_R])]
    sseq = [(d, 1) for d in s1[:LAG]] + [(d, 0) for d in small] + interleave(s0, s1[LAG:])
    cut = LAG + len(small) + 2 * n_m + 70

    issue(sseq[:cut])
    for d in small:
        d.wait()
    wait_all(wm_buf, S_M)
    c = c_buf[...].astype(f32)
    sc = (c * jax.nn.sigmoid(c)).astype(bf16)
    mod = jnp.dot(sc, wm_buf[...].reshape(D, 6 * D), preferred_element_type=f32)
    sa, ca, ga, sb, cb, gb = [mod[:, i * D:(i + 1) * D] for i in range(6)]
    x0 = x_buf[...].astype(f32)
    h1 = (_layernorm(x0) * (1.0 + ca) + sa).astype(bf16)

    issue_block(sseq[cut:])
    wait_all(wq_buf, S_Q)
    q = jnp.dot(h1, wq_buf[...].reshape(D, HQ * DH), preferred_element_type=f32)
    for hq in range(HQ):
        q_all[:, _qpos(hq), :] = q[:, hq * DH:(hq + 1) * DH]

    gu_specs = ((5, 4, 0, F, 512), (0, 5, 0, F, 384))
    e0 = wo_all[-n_late:] + wcopies(wg_hbm, wg_buf, S_G, *gu_specs)
    e1 = wcopies(wu_hbm, wu_buf, S_U, *gu_specs)
    n_g = len(e0)
    for j, (bl, bh, cl, ch, cw) in enumerate(STAGES):
        nb = (bh - bl) // 2
        if nb:
            e0 += wcopies(wd_hbm, wd_buf, S_D + j, (bl, nb, cl, ch, cw))
            e1 += wcopies(wd_hbm, wd_buf, S_D + j, (bl + nb, nb, cl, ch, cw))
        else:
            ps = wcopies(wd_hbm, wd_buf, S_D + j, (bl, 1, cl, ch, cw))
            e0 += ps[:len(ps) // 2]
            e1 += ps[len(ps) // 2:]
    e1 += [pltpu.make_async_copy(wo_hbm.at[0, pl.ds(0, 8), pl.ds(128 * j, 128)], pad_buf.at[j], sems.at[S_PAD])
           for j in range(LAG)]
    eseq = interleave(e0, e1[LV:])

    row_s = jax.lax.broadcasted_iota(jnp.int32, (QR, CH), 0) // 2
    row_o = jax.lax.broadcasted_iota(jnp.int32, (QR, DH), 0) // 2

    def group(t, carry):
        b = t // HPB
        q0 = pl.multiple_of((t % HPB) * QR, QR)
        qh = q_all[b, pl.ds(q0, QR), :].astype(bf16)

        def step(cidx, state):
            m, l, acc = state
            i = t * NC + cidx
            nxt = i + DK - 1

            @pl.when(nxt < NSTEP - 1)
            def _():
                issue(interleave(k_copies(nxt), v_copies(nxt)))

            @pl.when(nxt == NSTEP - 1)
            def _():
                issue(interleave(k_copies(NSTEP - 1), v_copies(NSTEP - 1, NPC - LV) + e1[:LV]))

            for e in range(DK - 1):
                @pl.when(nxt == NSTEP + e)
                def _():
                    issue(eseq[e * 2 * NPC:(e + 1) * 2 * NPC])

            ks = i % DK
            wait_all(kbuf.at[ks], S_K + ks)
            s = jax.lax.dot_general(qh, kbuf[ks, 0], NT, preferred_element_type=f32)
            for j in range(1, HG):
                sj = jax.lax.dot_general(qh, kbuf[ks, j], NT, preferred_element_type=f32)
                s = jnp.where(row_s == j, sj, s)
            m_new = jnp.maximum(m, jnp.max(s, axis=-1, keepdims=True))
            alpha = jnp.exp((m - m_new) * scale)
            p = jnp.exp((s - m_new) * scale)
            l = l * alpha + jnp.sum(p, axis=-1, keepdims=True)
            pb = p.astype(bf16)
            vs = i % DV
            wait_all(vbuf.at[vs], S_V + vs)
            o = jnp.dot(pb, vbuf[vs, 0], preferred_element_type=f32)
            for j in range(1, HG):
                oj = jnp.dot(pb, vbuf[vs, j], preferred_element_type=f32)
                o = jnp.where(row_o == j, oj, o)
            return m_new, l, acc * alpha + o

        init = (jnp.full((QR, 1), -jnp.inf, f32), jnp.zeros((QR, 1), f32), jnp.zeros((QR, DH), f32))
        _, l, acc = jax.lax.fori_loop(0, NC, step, init)
        o_all[b, pl.ds(q0, QR), :] = acc / l
        return carry

    jax.lax.fori_loop(0, NS, group, 0)

    p0 = (DK - 1) * 2 * NPC
    cuts = [p0, p0 + 40, p0 + 70, 2 * n_g + 70, 2 * n_g + 80, len(eseq)]

    issue_block(eseq[cuts[0]:cuts[1]])
    wait_all(wo_buf, S_O)
    parts = []
    for half in range(2):
        o_cat = jnp.concatenate([o_all[:, _qpos(half * (HQ // 2) + j), :] for j in range(HQ // 2)], axis=1)
        parts.append(jax.lax.dot_general(o_cat.astype(bf16),
                                         wo_buf[:, :, half * HW:(half + 1) * HW].reshape(D, HW), NT,
                                         preferred_element_type=f32))
        if half == 0:
            issue_block(eseq[cuts[1]:cuts[2]])
    x1 = x0 + ga * (parts[1] + parts[0])
    h2 = _layernorm(x1) * (1.0 + cb) + sb
    h2b = h2.astype(bf16)
    r = jnp.sum(h2 * wr_buf[...].astype(f32).reshape(1, D), axis=-1, keepdims=True)
    fin[0] = x1 + gb * h2
    fin[1] = gb * jax.nn.sigmoid(r)

    issue_block(eseq[cuts[2]:cuts[3]])
    wait_all(wg_buf, S_G)
    g = jnp.dot(h2b, wg_buf[...].reshape(D, F), preferred_element_type=f32)
    g = g * jax.nn.sigmoid(g)
    issue_block(eseq[cuts[3]:cuts[4]])
    wait_all(wu_buf, S_U)
    u = jnp.dot(h2b, wu_buf[...].reshape(D, F), preferred_element_type=f32)
    act = (g * u).astype(bf16)
    issue_block(eseq[cuts[4]:cuts[5]])

    n_early = STAGES[-1][0] * RB
    out_cps = [pltpu.make_async_copy(out_buf.at[:, pl.ds(c0, cn)], out_hbm.at[:, pl.ds(c0, cn)], sems.at[s])
               for c0, cn, s in ((0, n_early, S_OUT0), (n_early, D - n_early, S_OUT1))]
    for j, (bl, bh, cl, ch, _) in enumerate(STAGES):
        view = (pl.ds(bl, bh - bl), slice(None), pl.ds(cl, ch - cl))
        lo, hi = bl * RB, bh * RB
        wait_all(wd_buf.at[view], S_D + j)
        y = jax.lax.dot_general(act[:, cl:ch], wd_buf[view].reshape(hi - lo, ch - cl), NT,
                                preferred_element_type=f32)
        res = fin[0, :, lo:hi] + fin[1, :, lo:hi] * y
        if ch == F:
            out_buf[:, lo:hi] = res.astype(bf16)
            if hi == n_early:
                out_cps[0].start()
        else:
            fin[0, :, lo:hi] = res
    out_cps[1].start()
    wait_all(pad_buf, S_PAD)
    out_cps[0].wait()
    out_cps[1].wait()


@jax.jit
def pallas_adaLN_cond__sliding_block_cached__moe_arch_mod__decode_kernel(
    A_x: jax.Array,
    A_k_cache: jax.Array,
    A_v_cache: jax.Array,
    A_wq: jax.Array,
    A_wo: jax.Array,
    B_x: jax.Array,
    B_w_r: jax.Array,
    B_w_gate: jax.Array,
    B_w_up: jax.Array,
    B_w_down: jax.Array,
    c: jax.Array,
    w_mod: jax.Array,
):
    kv_shape = (B, HG, HPB, A_k_cache.shape[2], DH)
    out = pl.pallas_call(
        _kernel,
        out_shape=jax.ShapeDtypeStruct((B, D), bf16),
        in_specs=[pl.BlockSpec(memory_space=pl.ANY)] * 11,
        out_specs=pl.BlockSpec(memory_space=pl.ANY),
        scratch_shapes=[
            pltpu.VMEM((B, D), bf16), pltpu.VMEM((B, D), bf16), pltpu.VMEM((D,), bf16),
            pltpu.VMEM((NB_M, D // NB_M, 6 * D), bf16),
            pltpu.VMEM((NB, RB, HQ * DH), bf16), pltpu.VMEM((NB, RB, HQ * DH), bf16),
            pltpu.VMEM((NB, RB, F), bf16), pltpu.VMEM((NB, RB, F), bf16), pltpu.VMEM((NB, RB, F), bf16),
            pltpu.VMEM((LAG, 8, 128), bf16),
            pltpu.VMEM((DK, HG, CH, DH), bf16), pltpu.VMEM((DV, HG, CH, DH), bf16),
            pltpu.VMEM((B, HQ, DH), f32), pltpu.VMEM((B, HQ, DH), f32), pltpu.VMEM((2, B, D), f32),
            pltpu.VMEM((B, D), bf16),
            pltpu.SemaphoreType.DMA((S_V + DV,)),
        ],
        compiler_params=pltpu.CompilerParams(vmem_limit_bytes=64 * 1024 * 1024,
                                             disable_bounds_checks=True,
                                             disable_semaphore_checks=True),
    )(A_x.reshape(B, D), A_k_cache.reshape(kv_shape), A_v_cache.reshape(kv_shape),
      A_wq.reshape(NB, RB, HQ * DH), A_wo.T.reshape(NB, RB, HQ * DH), B_w_r,
      B_w_gate.reshape(NB, RB, F), B_w_up.reshape(NB, RB, F), B_w_down.T.reshape(NB, RB, F),
      c, w_mod.reshape(NB_M, D // NB_M, 6 * D))
    return out.reshape(B, 1, D)
```

```python
import jax
import jax.numpy as jnp
import jax.experimental.pallas as pl
import jax.experimental.pallas.tpu as pltpu

B, D = 8, 576
HQ, HKV, DH = 32, 16, 128
F = 4608
EPS = 1e-05
NT = (((1,), (1,)), ((), ()))
f32 = jnp.float32
bf16 = jnp.bfloat16

HG, CH, R = 8, 512, 16
NPC = CH // R
QR = 2 * HG
NW = B * HKV
NG = NW // HG // 2
LAG = 26
W0R = 128
D0 = 2
D1 = D0 + 1
NB_M, NB = 4, 9
RB = D // NB
HW = HQ * DH // 2
CS = 3072
STAGES = ((0, 6, 0, F, 768), (6, 8, 0, F, F // 2), (8, 9, 0, CS, CS), (8, 9, CS, F, F - CS))
S_C, S_X, S_R, S_PAD, S_M, S_Q, S_O, S_G, S_U, S_OUT0, S_OUT1, S_W0, S_D = range(13)
S_KV = S_D + len(STAGES)
S_RING = (S_KV, S_KV + D0, S_KV + 2 * D0, S_KV + 2 * D0 + D1)
N_SEM = S_KV + 2 * D0 + 2 * D1


def _layernorm(x):
    m = jnp.mean(x, axis=-1, keepdims=True)
    xc = x - m
    v = jnp.mean(xc * xc, axis=-1, keepdims=True)
    return xc / jnp.sqrt(v + EPS)


def _kernel(x_hbm, k_hbm, v_hbm, wq_hbm, wo_hbm, wr_hbm, wg_hbm, wu_hbm, wd_hbm, c_hbm, wm_hbm,
            out_hbm,
            x_buf, c_buf, wr_buf, wm_buf, wq_buf, wo_buf, wg_buf, wu_buf, wd_buf, pad_buf,
            k0buf, v0buf, k1buf, v1buf, w0buf, q_all, o_all, fin, out_buf, sems):
    SK = k_hbm.shape[1]
    W = w0buf.shape[1]
    NC = W // CH
    NSTEP = NG * NC
    rings = (k0buf, v0buf, k1buf, v1buf)
    scale = DH ** -0.5

    def wcopies(src, dst, s, *specs):
        out = []
        for b0, nb, c_lo, c_hi, cw in specs:
            for r in range(0, src.shape[1], 8):
                for c0 in range(c_lo, c_hi, cw):
                    idx = (pl.ds(b0, nb), pl.ds(r, 8), pl.ds(c0, min(cw, c_hi - c0)))
                    out.append(pltpu.make_async_copy(src.at[idx], dst.at[idx], sems.at[s]))
        return out

    def kv_copies(qu, i, last=False, lo=0, hi=2 * NPC):
        r0 = SK - W + (i % NC) * CH
        w0, nw = (NW - HG + 1, HG - 1) if last else ((i // NC + qu * NG) * HG + 1, HG)
        out = []
        for n in range(lo, hi):
            a, c = n // NPC, n % NPC * R
            buf = rings[2 * qu + a]
            slot = i % buf.shape[0]
            out.append(pltpu.make_async_copy(
                (k_hbm, v_hbm)[a].at[pl.ds(w0, nw), pl.ds(pl.multiple_of(r0 + c, R), R), :],
                buf.at[slot, pl.ds(0, nw), pl.ds(c, R), :], sems.at[S_RING[2 * qu + a] + slot]))
        return out

    def interleave(l0, l1):
        assert len(l0) == len(l1)
        return [x for d0, d1 in zip(l0, l1) for x in ((d0, 0), (d1, 1))]

    def issue(seq):
        for d, prio in seq:
            d.start(priority=prio)

    def issue_block(seq):
        half = (len(seq) + 1) // 2

        def body(it, carry):
            @pl.when(it == 0)
            def _():
                issue(seq[:half])

            @pl.when(it == 1)
            def _():
                issue(seq[half:])
            return carry

        jax.lax.fori_loop(0, 2, body, 0)

    def wait_all(buf, s):
        pltpu.make_async_copy(buf, buf, sems.at[s]).wait()

    qo_specs = ((0, 1, 0, 2 * HW, HW), (1, 8, 0, 2 * HW, 256))
    s0 = wcopies(wm_hbm, wm_buf, S_M, (0, 2, 0, 6 * D, 1152))
    s1 = wcopies(wm_hbm, wm_buf, S_M, (2, 2, 0, 6 * D, 1152))
    n_m = len(s0)
    s0 += wcopies(wo_hbm, wo_buf, S_O, *qo_specs)
    s1 += wcopies(wq_hbm, wq_buf, S_Q, *qo_specs)
    n_q = len(s0)
    for lst, src, a in ((s0, k_hbm, 0), (s1, v_hbm, 1)):
        lst += [pltpu.make_async_copy(src.at[0, pl.ds(SK - W + r, W0R), :], w0buf.at[a, pl.ds(r, W0R), :],
                                      sems.at[S_W0]) for r in range(0, W, W0R)]
    for i in range(D0 - 1):
        s0 += kv_copies(0, i)
        s1 += kv_copies(1, i)
    s1 += kv_copies(1, D0 - 1, False, 0, LAG)
    small = [pltpu.make_async_copy(c_hbm, c_buf, sems.at[S_C]),
             pltpu.make_async_copy(x_hbm, x_buf, sems.at[S_X]),
             pltpu.make_async_copy(wr_hbm, wr_buf, sems.at[S_R])]
    sseq = [(d, 1) for d in s1[:LAG]] + [(d, 0) for d in small] + interleave(s0, s1[LAG:])
    cut = LAG + len(small) + 2 * n_m + 70
    cut_q = LAG + len(small) + 2 * n_q + 70

    issue(sseq[:cut])
    for d in small:
        d.wait()
    wait_all(wm_buf, S_M)
    c = c_buf[...].astype(f32)
    sc = (c * jax.nn.sigmoid(c)).astype(bf16)
    mod = jnp.dot(sc, wm_buf[...].reshape(D, 6 * D), preferred_element_type=f32)
    sa, ca, ga, sb, cb, gb = [mod[:, i * D:(i + 1) * D] for i in range(6)]
    x0 = x_buf[...].astype(f32)
    h1 = (_layernorm(x0) * (1.0 + ca) + sa).astype(bf16)

    issue_block(sseq[cut:cut_q])
    wait_all(wq_buf, S_Q)
    q = jnp.dot(h1, wq_buf[...].reshape(D, HQ * DH), preferred_element_type=f32)
    for hq in range(HQ):
        qc = q[:, hq * DH:(hq + 1) * DH]
        q_all[:, (hq - 2) % HQ, :] = qc if hq >= 2 else jnp.concatenate([qc[1:], qc[:1]], axis=0)
    issue_block(sseq[cut_q:])
    wait_all(w0buf, S_W0)

    gu_specs = ((5, 4, 0, F, 512), (0, 5, 0, F, 384))
    e0 = wcopies(wg_hbm, wg_buf, S_G, *gu_specs)
    e1 = wcopies(wu_hbm, wu_buf, S_U, *gu_specs)
    n_g = len(e0)
    for j, (bl, bh, cl, ch, cw) in enumerate(STAGES):
        nb = (bh - bl) // 2
        if nb:
            e0 += wcopies(wd_hbm, wd_buf, S_D + j, (bl, nb, cl, ch, cw))
            e1 += wcopies(wd_hbm, wd_buf, S_D + j, (bl + nb, nb, cl, ch, cw))
        else:
            ps = wcopies(wd_hbm, wd_buf, S_D + j, (bl, 1, cl, ch, cw))
            e0 += ps[:len(ps) // 2]
            e1 += ps[len(ps) // 2:]
    e1 += [pltpu.make_async_copy(wo_hbm.at[0, pl.ds(0, 8), pl.ds(128 * j, 128)], pad_buf.at[j], sems.at[S_PAD])
           for j in range(LAG)]
    eseq = interleave(e0, e1[LAG:])

    row_s = jax.lax.broadcasted_iota(jnp.int32, (QR, CH), 0) // 2
    row_o = jax.lax.broadcasted_iota(jnp.int32, (QR, DH), 0) // 2

    n_tail = 80

    def group(t, carry):
        rows = [(t // 2 + qu * (B // 2), pl.ds(pl.multiple_of((t % 2) * QR, QR), QR)) for qu in range(2)]
        qh = [q_all[b, ds, :].astype(bf16) for b, ds in rows]

        def step(cidx, state):
            i = t * NC + cidx
            nxt = i + D0 - 1
            first_last = NSTEP - NC

            @pl.when(nxt < first_last - 1)
            def _():
                issue(interleave(kv_copies(0, nxt),
                                 kv_copies(1, nxt, False, LAG) + kv_copies(1, nxt + 1, False, 0, LAG)))

            @pl.when(nxt == first_last - 1)
            def _():
                n = first_last - 1
                issue(interleave(kv_copies(0, n),
                                 kv_copies(1, n, False, LAG) + kv_copies(1, n + 1, True, 0, LAG)))

            @pl.when(jnp.logical_and(nxt >= first_last, nxt < NSTEP - 1))
            def _():
                issue(interleave(kv_copies(0, nxt),
                                 kv_copies(1, nxt, True, LAG) + kv_copies(1, nxt + 1, True, 0, LAG)))

            @pl.when(nxt == NSTEP - 1)
            def _():
                issue(interleave(kv_copies(0, NSTEP - 1), kv_copies(1, NSTEP - 1, True, LAG) + e1[:LAG]))

            for e in range(D0 - 1):
                @pl.when(nxt == NSTEP + e)
                def _():
                    issue(eseq[e * n_tail:(e + 1) * n_tail])

            slots = [i % buf.shape[0] for buf in rings]

            def wait_chunks(a):
                wait_all(rings[a].at[slots[a]], S_RING[a] + slots[a])
                buf, slot = rings[2 + a], slots[2 + a]

                @pl.when(t < NG - 1)
                def _():
                    wait_all(buf.at[slot], S_RING[2 + a] + slot)

                @pl.when(t == NG - 1)
                def _():
                    wait_all(buf.at[slot, pl.ds(0, HG - 1)], S_RING[2 + a] + slot)
                    buf[slot, HG - 1] = w0buf[a, pl.ds(pl.multiple_of(cidx * CH, CH), CH), :]

            wait_chunks(0)
            mid = []
            for qu in range(2):
                m, l, _ = state[qu]
                kb, ks = rings[2 * qu], slots[2 * qu]
                s = jax.lax.dot_general(qh[qu], kb[ks, 0], NT, preferred_element_type=f32)
                for j in range(1, HG):
                    sj = jax.lax.dot_general(qh[qu], kb[ks, j], NT, preferred_element_type=f32)
                    s = jnp.where(row_s == j, sj, s)
                m_new = jnp.maximum(m, jnp.max(s, axis=-1, keepdims=True))
                alpha = jnp.exp((m - m_new) * scale)
                p = jnp.exp((s - m_new) * scale)
                mid.append((m_new, l * alpha + jnp.sum(p, axis=-1, keepdims=True), alpha, p.astype(bf16)))
            wait_chunks(1)
            new = []
            for qu in range(2):
                m_new, l, alpha, pb = mid[qu]
                vb, vs = rings[2 * qu + 1], slots[2 * qu + 1]
                o = jnp.dot(pb, vb[vs, 0], preferred_element_type=f32)
                for j in range(1, HG):
                    oj = jnp.dot(pb, vb[vs, j], preferred_element_type=f32)
                    o = jnp.where(row_o == j, oj, o)
                new.append((m_new, l, state[qu][2] * alpha + o))
            return tuple(new)

        init = (jnp.full((QR, 1), -jnp.inf, f32), jnp.zeros((QR, 1), f32), jnp.zeros((QR, DH), f32))
        state = jax.lax.fori_loop(0, NC, step, (init, init))
        for (b, ds), (_, l, acc) in zip(rows, state):
            o_all[b, ds, :] = acc / l
        return carry

    jax.lax.fori_loop(0, NG, group, 0)

    p0 = (D0 - 1) * n_tail
    cuts = [p0, p0 + 40, p0 + 70, 2 * n_g + 70, 2 * n_g + 80, len(eseq)]

    issue_block(eseq[cuts[0]:cuts[1]])
    wait_all(wo_buf, S_O)
    parts = []
    for half in range(2):
        cols = [o_all[:, (hq - 2) % HQ, :] for hq in range(half * (HQ // 2), (half + 1) * (HQ // 2))]
        if half == 0:
            cols[:2] = [jnp.concatenate([oc[B - 1:], oc[:B - 1]], axis=0) for oc in cols[:2]]
        o_cat = jnp.concatenate(cols, axis=1)
        parts.append(jax.lax.dot_general(o_cat.astype(bf16),
                                         wo_buf[:, :, half * HW:(half + 1) * HW].reshape(D, HW), NT,
                                         preferred_element_type=f32))
        if half == 0:
            issue_block(eseq[cuts[1]:cuts[2]])
    x1 = x0 + ga * (parts[1] + parts[0])
    h2 = _layernorm(x1) * (1.0 + cb) + sb
    h2b = h2.astype(bf16)
    r = jnp.sum(h2 * wr_buf[...].astype(f32).reshape(1, D), axis=-1, keepdims=True)
    fin[0] = x1 + gb * h2
    fin[1] = gb * jax.nn.sigmoid(r)

    issue_block(eseq[cuts[2]:cuts[3]])
    wait_all(wg_buf, S_G)
    g = jnp.dot(h2b, wg_buf[...].reshape(D, F), preferred_element_type=f32)
    g = g * jax.nn.sigmoid(g)
    issue_block(eseq[cuts[3]:cuts[4]])
    wait_all(wu_buf, S_U)
    u = jnp.dot(h2b, wu_buf[...].reshape(D, F), preferred_element_type=f32)
    act = (g * u).astype(bf16)
    issue_block(eseq[cuts[4]:cuts[5]])

    n_early = STAGES[-1][0] * RB
    out_cps = [pltpu.make_async_copy(out_buf.at[:, pl.ds(c0, cn)], out_hbm.at[:, pl.ds(c0, cn)], sems.at[s])
               for c0, cn, s in ((0, n_early, S_OUT0), (n_early, D - n_early, S_OUT1))]
    for j, (bl, bh, cl, ch, _) in enumerate(STAGES):
        view = (pl.ds(bl, bh - bl), slice(None), pl.ds(cl, ch - cl))
        lo, hi = bl * RB, bh * RB
        wait_all(wd_buf.at[view], S_D + j)
        y = jax.lax.dot_general(act[:, cl:ch], wd_buf[view].reshape(hi - lo, ch - cl), NT,
                                preferred_element_type=f32)
        res = fin[0, :, lo:hi] + fin[1, :, lo:hi] * y
        if ch == F:
            out_buf[:, lo:hi] = res.astype(bf16)
            if hi == n_early:
                out_cps[0].start()
        else:
            fin[0, :, lo:hi] = res
    out_cps[1].start()
    wait_all(pad_buf, S_PAD)
    out_cps[0].wait()
    out_cps[1].wait()


@jax.jit
def pallas_adaLN_cond__sliding_block_cached__moe_arch_mod__decode_kernel(
    A_x: jax.Array,
    A_k_cache: jax.Array,
    A_v_cache: jax.Array,
    A_wq: jax.Array,
    A_wo: jax.Array,
    B_x: jax.Array,
    B_w_r: jax.Array,
    B_w_gate: jax.Array,
    B_w_up: jax.Array,
    B_w_down: jax.Array,
    c: jax.Array,
    w_mod: jax.Array,
):
    kv_shape = (NW, A_k_cache.shape[2], DH)
    window = min(4096, max(256, A_k_cache.shape[2] // 4))
    out = pl.pallas_call(
        _kernel,
        out_shape=jax.ShapeDtypeStruct((B, D), bf16),
        in_specs=[pl.BlockSpec(memory_space=pl.ANY)] * 11,
        out_specs=pl.BlockSpec(memory_space=pl.ANY),
        scratch_shapes=[
            pltpu.VMEM((B, D), bf16), pltpu.VMEM((B, D), bf16), pltpu.VMEM((D,), bf16),
            pltpu.VMEM((NB_M, D // NB_M, 6 * D), bf16),
            pltpu.VMEM((NB, RB, HQ * DH), bf16), pltpu.VMEM((NB, RB, HQ * DH), bf16),
            pltpu.VMEM((NB, RB, F), bf16), pltpu.VMEM((NB, RB, F), bf16), pltpu.VMEM((NB, RB, F), bf16),
            pltpu.VMEM((LAG, 8, 128), bf16),
            pltpu.VMEM((D0, HG, CH, DH), bf16), pltpu.VMEM((D0, HG, CH, DH), bf16),
            pltpu.VMEM((D1, HG, CH, DH), bf16), pltpu.VMEM((D1, HG, CH, DH), bf16),
            pltpu.VMEM((2, window, DH), bf16),
            pltpu.VMEM((B, HQ, DH), f32), pltpu.VMEM((B, HQ, DH), f32), pltpu.VMEM((2, B, D), f32),
            pltpu.VMEM((B, D), bf16),
            pltpu.SemaphoreType.DMA((N_SEM,)),
        ],
        compiler_params=pltpu.CompilerParams(vmem_limit_bytes=64 * 1024 * 1024,
                                             disable_bounds_checks=True,
                                             disable_semaphore_checks=True),
    )(A_x.reshape(B, D), A_k_cache.reshape(kv_shape), A_v_cache.reshape(kv_shape),
      A_wq.reshape(NB, RB, HQ * DH), A_wo.T.reshape(NB, RB, HQ * DH), B_w_r,
      B_w_gate.reshape(NB, RB, F), B_w_up.reshape(NB, RB, F), B_w_down.T.reshape(NB, RB, F),
      c, w_mod.reshape(NB_M, D // NB_M, 6 * D))
    return out.reshape(B, 1, D)
```
